```python
import os as _os
_os.environ.setdefault("JAX_PLATFORMS", "cpu")
import jax
import jax.numpy as jnp

def _softmax(x, axis=-1):
    return jax.nn.softmax(x, axis=axis)
def _gelu(x):
    return jax.nn.gelu(x, approximate=True)
def _silu(x):
    return jax.nn.silu(x)
def _sigmoid(x):
    return jax.nn.sigmoid(x)
def _layernorm(x, axis=-1, eps=1e-5):
    m = jnp.mean(x, axis=axis, keepdims=True)
    v = jnp.var(x, axis=axis, keepdims=True)
    return (x - m) / jnp.sqrt(v + eps)
def _scatter_add(tgt, idx, src, axis=0):
    return tgt.at[idx].add(src)
def _segment_sum(src, seg, n):
    return jax.ops.segment_sum(src, seg, n)
class _Rng:
    def __init__(self, key):
        self._k = key
    def _next(self):
        self._k, sub = jax.random.split(self._k)
        return sub
    def normal(self, shape):
        return jax.random.normal(self._next(), shape, dtype=jnp.bfloat16)
    def randint(self, lo, hi, shape):
        return jax.random.randint(self._next(), shape, lo, hi, dtype=jnp.int32)
    def uniform(self, shape, lo=0.0, hi=1.0):
        return jax.random.uniform(self._next(), shape, jnp.bfloat16, lo, hi)
    def permutation(self, n):
        return jax.random.permutation(self._next(), n)


kernel_name = 'sequential_preLN__sliding_block__glu_gated_swiglu__prompt'

def setup_inputs():
    _rng = _Rng(jax.random.key(int.from_bytes(__import__("os").urandom(4), "little")))
    _w = (lambda a: (lambda t: t.astype(jnp.bfloat16) if jnp.issubdtype(t.dtype, jnp.floating) else t)(jnp.asarray(a)))
    def _A_setup():
        B, S, D = 1, 2048, 640
        return {
            "x": _w((lambda *s: _rng.normal(s) * 0.05)(B, S, D)),
            "wqkv": _w((lambda *s: _rng.normal(s) * 0.05)(D, 3 * D)),
            "wo": _w((lambda *s: _rng.normal(s) * 0.05)(D, D)),
        }
    _A_in = _A_setup()

    def _B_setup():
        B, S, D, F = 1, 2048, 640, 1728
        return {
            "x": _w((lambda *s: _rng.normal(s) * 0.05)(B, S, D)),
            "w1": _w((lambda *s: _rng.normal(s) * 0.1)(D, F) * (2.0 / D) ** 0.5),
            "w3": _w((lambda *s: _rng.normal(s) * 0.1)(D, F) * (2.0 / D) ** 0.5),
            "w2": _w((lambda *s: _rng.normal(s) * 0.1)(F, D) * (2.0 / F) ** 0.5),
        }
    _B_in = _B_setup()

    return {
        "A_x": _A_in["x"],
        "A_wqkv": _A_in["wqkv"],
        "A_wo": _A_in["wo"],
        "B_x": _B_in["x"],
        "B_w1": _B_in["w1"],
        "B_w3": _B_in["w3"],
        "B_w2": _B_in["w2"],
    }

def reference(A_x, A_wqkv, A_wo, B_x, B_w1, B_w3, B_w2):
    def _A_ref(x, wqkv, wo):
        B, S, D = x.shape
        H = 32; Dh = D // H; W = 256
        qkv = (lambda x, *d: x.transpose(*d))((x @ wqkv).reshape(B, S, 3, H, Dh), 2, 0, 3, 1, 4)
        q, k, v = qkv[0], qkv[1], qkv[2]
        scores = jnp.einsum("bhqd,bhkd->bhqk", q, k) * (Dh ** -0.5)
        idx = jnp.arange(S)
        mask = (idx[:, None] - idx[None, :] >= 0) & (idx[:, None] - idx[None, :] < W)
        scores = jnp.where(mask[None, None], scores, -1e9)
        p = _softmax(scores, axis=-1)
        o = jnp.einsum("bhqk,bhkd->bhqd", p, v)
        return (lambda x, *d: x.transpose(*d))(o, 0, 2, 1, 3).reshape(B, S, D) @ wo

    def _B_ref(x, w1, w3, w2):
        gate = jnp.einsum("bsd,df->bsf", x, w1)
        up = jnp.einsum("bsd,df->bsf", x, w3)
        h = _silu(gate) * up
        out = jnp.einsum("bsf,fd->bsd", h, w2)
        return out

    x = A_x
    h = x + _A_ref(_layernorm(x, axis=-1), A_wqkv, A_wo)
    h2 = h + _B_ref(_layernorm(h, axis=-1), B_w1, B_w3, B_w2)
    return h2
```

```python
import functools
import jax
import jax.numpy as jnp
import jax.experimental.pallas as pl
import jax.experimental.pallas.tpu as pltpu

S, D, F = 2048, 640, 1728
H, DH, W = 32, 20, 256
NG = 8
LOG2E = 1.4426950408889634
NEG = -1e30
f32 = jnp.float32
bf16 = jnp.bfloat16
i32 = jnp.int32
NT = (((1,), (1,)), ((), ()))
ONES_PK = 0x3F803F80
T = 256
NQ = T // 128
NB = S // T


def _ln(x):
    m = jnp.mean(x, axis=-1, keepdims=True)
    xc = x - m
    v = jnp.mean(xc * xc, axis=-1, keepdims=True)
    return xc * jax.lax.rsqrt(v + 1e-5)


def _group_tile(a, g):
    lo = 80 * g
    t0, off = lo // 128, lo % 128
    ta = a[:, t0 * 128:(t0 + 1) * 128]
    if off + 80 <= 128:
        return ta
    tb = a[:, (t0 + 1) * 128:(t0 + 2) * 128]
    lane = jax.lax.broadcasted_iota(i32, ta.shape, 1)
    return jnp.where(lane >= off, ta, tb)


def _pack(a):
    n = a.shape[0] // 16
    outs = [pltpu.pack_elementwise([a[16 * t:16 * t + 8], a[16 * t + 8:16 * t + 16]], packed_dtype=bf16)
            for t in range(n)]
    o = jnp.concatenate(outs, axis=0) if n > 1 else outs[0]
    return o.astype(i32) if o.dtype != i32 else o


def _silu(g):
    return g * (0.5 * jnp.tanh(0.5 * g) + 0.5)


def make(DEPTH0=2, DEPTH=0, ORDER=0):

    def attn_fns(first, tok, q_ref, k_ref, vt_ref, ot_ref, s_ref):
        lane16 = jax.lax.broadcasted_iota(i32, (16, 128), 1)
        row16 = jax.lax.broadcasted_iota(i32, (16, 128), 0)
        lane32 = jax.lax.broadcasted_iota(i32, (32, 128), 1)
        row32 = jax.lax.broadcasted_iota(i32, (32, 128), 0)
        tri = row32 <= (lane32 % 32)
        b0 = (lane16 & 32) == 0
        b1 = (lane16 & 64) == 0
        b0_24 = (jax.lax.broadcasted_iota(i32, (24, 128), 1) & 32) == 0
        zero16 = jnp.zeros((16, 128), i32)

        def info(qb):
            return (8 - 4 * qb) if first else 0

        def qk(slot, qb, g):
            miss = info(qb)
            masks = []
            for h in range(4):
                lo = (80 * g + 20 * h) % 128
                if lo + 20 <= 128:
                    msk = (lane16 >= lo) & (lane16 < lo + 20)
                else:
                    msk = (lane16 >= lo) | (lane16 < lo + 20 - 128)
                masks.append(jnp.where(msk, -1, 0))
            mxs = []
            for j in range(4):
                q = q_ref[g, qb * 64 + 16 * j: qb * 64 + 16 * j + 16, :]
                wq = pltpu.bitcast(jnp.concatenate([q & masks[m ^ j] for m in range(4)], axis=0), bf16)
                c0 = max(j, miss)
                c1 = j + 9
                nrows = (c1 - c0) * 32
                if first:
                    r0 = qb * 64 + 16 * c0
                    kk = k_ref[g, r0: r0 + nrows // 2, :]
                else:
                    kk = k_ref[g, pl.ds(pl.multiple_of(tok // 2 + qb * 64 + 16 * c0, 16), nrows // 2), :]
                s = jax.lax.dot_general(pltpu.bitcast(kk, bf16), wq, NT, preferred_element_type=f32)
                bot = s[nrows - 32:, :]
                if c0 == j:
                    sm = jnp.where(tri, bot, s[:32, :])
                    mid = s[32:nrows - 32, :]
                else:
                    sm = jnp.where(tri, bot, NEG)
                    mid = s[:nrows - 32, :] if nrows > 32 else None
                allm = sm if mid is None else jnp.concatenate([mid, sm], axis=0)
                n = allm.shape[0]
                s_ref[slot, j, 256 - n:, :] = allm
                parts = [allm[8 * t:8 * t + 8] for t in range(n // 8)]
                accs = parts[:4]
                for t in range(4, len(parts)):
                    accs[t % 4] = jnp.maximum(accs[t % 4], parts[t])
                m8 = jnp.maximum(jnp.maximum(accs[0], accs[1]), jnp.maximum(accs[2], accs[3]))
                mx = jnp.max(m8, axis=0, keepdims=True)
                mxs.append(jnp.broadcast_to(mx, (32, 128)))
            return mxs

        def softpv(slot, qb, g, mxs):
            miss = info(qb)
            pm = [jnp.exp2(s_ref[slot, j, 224:256, :] - mxs[j]) for j in range(4)]
            Z = [[] for _ in range(4)]
            for c in range(miss, 12):
                X = []
                for j in range(4):
                    if c < j or c > j + 8:
                        X.append(None)
                    elif c == j:
                        X.append(_pack(jnp.where(tri, 0.0, pm[j])))
                    elif c == j + 8:
                        X.append(_pack(jnp.where(tri, pm[j], 0.0)))
                    else:
                        cc = c - j - 1
                        X.append(_pack(jnp.exp2(s_ref[slot, j, 32 * cc:32 * cc + 32, :] - mxs[j])))

                def sel(mask, a, b):
                    if a is None and b is None:
                        return None
                    return jnp.where(mask, zero16 if a is None else a, zero16 if b is None else b)
                Y = [[sel(b0, X[2 * j1], X[2 * j1 + 1]), sel(b0, X[2 * j1 + 1], X[2 * j1])] for j1 in range(2)]
                for h0 in range(2):
                    Z[h0].append(sel(b1, Y[0][h0], Y[1][h0]))
                    Z[2 + h0].append(sel(b1, Y[1][h0], Y[0][h0]))
            outs = []
            for h in range(4):
                hh = 4 * g + h
                ph = pltpu.bitcast(jnp.concatenate(Z[h], axis=0), bf16)
                w0 = (20 * hh) // 16 * 16
                o = 20 * hh - w0
                t0 = miss // 4
                vts = []
                for t in range(t0, 3):
                    if first:
                        v = vt_ref[qb + t, w0 // 2:w0 // 2 + 16, :]
                    else:
                        v = vt_ref[tok // 128 + qb + t, w0 // 2:w0 // 2 + 16, :]
                    ones_rows = (row16 >= 12) if o < 8 else (row16 < 4)
                    vts.append(jnp.where(ones_rows, ONES_PK, v))
                vt = pltpu.bitcast(jnp.concatenate(vts, axis=1) if len(vts) > 1 else vts[0], bf16)
                r = jnp.dot(vt, ph, preferred_element_type=f32)
                if o < 8:
                    l8, dat = r[24:32, :], r[0:24, :]
                else:
                    l8, dat = r[0:8, :], r[8:32, :]
                inv = pl.reciprocal(l8, approx=True)
                inv = inv * (2.0 - l8 * inv)
                dat = dat * jnp.concatenate([inv, inv, inv], axis=0)
                if h == 1:
                    dat = jnp.where(b0_24, pltpu.roll(dat, 96, 1), pltpu.roll(dat, 32, 1))
                elif h == 2:
                    dat = pltpu.roll(dat, 64, 1)
                elif h == 3:
                    dat = jnp.where(b0_24, pltpu.roll(dat, 32, 1), pltpu.roll(dat, 96, 1))
                outs.append(dat)
            sub = jax.lax.broadcasted_iota(i32, (8, 128), 0)
            og = jnp.concatenate([
                outs[0][0:16], jnp.where(sub < 4, outs[0][16:24], outs[1][0:8]), outs[1][8:24],
                outs[2][0:16], jnp.where(sub < 4, outs[2][16:24], outs[3][0:8]), outs[3][8:24]], axis=0)
            ot_ref[qb, 80 * g:80 * g + 80, :] = og
        return qk, softpv

    def kern(x_ref, wqkv_hbm, wo_hbm, w1t_hbm, w3t_hbm, w2_hbm, o_ref,
             wqkv_ref, wvt_ref, wo_ref, w13_ref, w2_ref, q_ref, k_ref, vt_ref, ot_ref, s_ref,
             h_ref, hn_ref, sems):
        i = pl.program_id(0)

        def copies():
            return [pltpu.make_async_copy(wqkv_hbm.at[:, 0:D], wqkv_ref.at[:, 0:D], sems.at[0]),
                    pltpu.make_async_copy(wqkv_hbm.at[:, D:2 * D], wqkv_ref.at[:, D:2 * D], sems.at[1]),
                    pltpu.make_async_copy(wqkv_hbm.at[:, 2 * D:], wqkv_ref.at[:, 2 * D:], sems.at[2]),
                    pltpu.make_async_copy(wo_hbm, wo_ref, sems.at[3]),
                    pltpu.make_async_copy(w1t_hbm, w13_ref.at[0], sems.at[4]),
                    pltpu.make_async_copy(w3t_hbm, w13_ref.at[1], sems.at[5]),
                    pltpu.make_async_copy(w2_hbm, w2_ref, sems.at[6])]

        def ffn_pieces():
            st = {}
            acts = []

            def up(c):
                def run():
                    if 'hn' not in st:
                        st['hn'] = pltpu.bitcast(hn_ref[...], bf16)
                    hn = st['hn']
                    if c < 13:
                        gt = jax.lax.dot_general(hn, w13_ref[0, 128 * c:128 * c + 128, :], NT, preferred_element_type=f32)
                        u = jax.lax.dot_general(hn, w13_ref[1, 128 * c:128 * c + 128, :], NT, preferred_element_type=f32)
                        acts.append((_silu(gt) * u).astype(bf16))
                    else:
                        wl = jnp.concatenate([w13_ref[0, 1664:1728, :], w13_ref[1, 1664:1728, :]], axis=0)
                        gu = jax.lax.dot_general(hn, wl, NT, preferred_element_type=f32)
                        a = _silu(gu) * pltpu.roll(gu, 64, 1)
                        acts.append(a[:, :64].astype(bf16))
                return run

            def down(n):
                def run():
                    if 'a' not in st:
                        st['a'] = jnp.concatenate(acts, axis=1)
                    r = jnp.dot(st['a'], w2_ref[:, 128 * n:128 * n + 128], preferred_element_type=f32)
                    o_ref[:, 128 * n:128 * n + 128] = (h_ref[:, 128 * n:128 * n + 128] + r).astype(bf16)
                return run
            return [up(c) for c in range(14)] + [down(n) for n in range(5)]

        def body(doA, doB, first):
            pieces = ffn_pieces() if doB else []

            def piece():
                if pieces:
                    pieces.pop(0)()
            if not doA:
                while pieces:
                    piece()
                return
            if first:
                cs = copies()
                for c in cs[:3]:
                    c.start()
            piece()
            x = x_ref[...].astype(f32)
            xnf = _ln(x)
            xn = xnf.astype(bf16)
            xnv = pltpu.bitcast(_pack(xnf), bf16)
            tok = 0 if first else pl.multiple_of(i * T, T)
            if first:
                cs[0].wait()
            q = jnp.dot(xn, wqkv_ref[:, :D], preferred_element_type=f32)
            q = pltpu.bitcast((q * (DH ** -0.5 * LOG2E)).astype(bf16), i32)
            for g in range(NG):
                q_ref[g] = _group_tile(q, g)
            if first:
                cs[1].wait()
            k = jnp.dot(xn, wqkv_ref[:, D:2 * D], preferred_element_type=f32)
            k = pltpu.bitcast(k.astype(bf16), i32)
            for g in range(NG):
                kg = _group_tile(k, g)
                if first:
                    k_ref[g, W // 2:W // 2 + T // 2, :] = kg
                else:
                    k_ref[g, pl.ds(pl.multiple_of(W // 2 + tok // 2, T // 2), T // 2), :] = kg
            if first:
                cs[2].wait()
                for c in cs[3:]:
                    c.start()
                wvt_ref[...] = wqkv_ref[:, 2 * D:].astype(f32).T.astype(bf16)
            vt = jax.lax.dot_general(wvt_ref[...], xnv, NT, preferred_element_type=f32).astype(bf16)
            vt = pltpu.bitcast(vt, i32)
            for t in range(NQ):
                if first:
                    vt_ref[2 + t] = vt[:, t * 128:(t + 1) * 128]
                else:
                    vt_ref[2 + i * NQ + t] = vt[:, t * 128:(t + 1) * 128]
            qk, softpv = attn_fns(first, tok, q_ref, k_ref, vt_ref, ot_ref, s_ref)
            items = [(qb, g) for qb in range(NQ) for g in range(NG)]
            n = len(items)
            dep = DEPTH if doB else DEPTH0
            NS = dep + 1
            ss = {}
            for t in range(min(dep, n)):
                ss[t] = qk(t % NS, *items[t])
            for t in range(n):
                if t + dep < n:
                    ss[t + dep] = qk((t + dep) % NS, *items[t + dep])
                piece()
                softpv(t % NS, *items[t], ss.pop(t))
            piece()
            o = jnp.concatenate([ot_ref[qb].T for qb in range(NQ)], axis=0).astype(bf16)
            if first:
                cs[3].wait()
            h = x + jnp.dot(o, wo_ref[...], preferred_element_type=f32)
            piece()
            assert not pieces
            h_ref[...] = h
            hn_ref[...] = pltpu.bitcast(_ln(h).astype(bf16), i32)
            if first:
                for c in cs[4:]:
                    c.wait()

        @pl.when(i == 0)
        def _():
            body(True, False, True)

        @pl.when((i > 0) & (i < NB))
        def _():
            body(True, True, False)

        @pl.when(i == NB)
        def _():
            body(False, True, False)

    @jax.jit
    def f(A_x, A_wqkv, A_wo, B_x, B_w1, B_w3, B_w2):
        x = A_x.reshape(S, D)
        anyspec = pl.BlockSpec(memory_space=pl.ANY)
        out = pl.pallas_call(
            kern,
            out_shape=jax.ShapeDtypeStruct((S, D), bf16),
            grid=(NB + 1,),
            in_specs=[pl.BlockSpec((T, D), lambda i: (jnp.minimum(i, NB - 1), 0))] + [anyspec] * 5,
            out_specs=pl.BlockSpec((T, D), lambda i: (jnp.maximum(i - 1, 0), 0)),
            scratch_shapes=[
                pltpu.VMEM((D, 3 * D), bf16),
                pltpu.VMEM((D, D), bf16),
                pltpu.VMEM((D, D), bf16),
                pltpu.VMEM((2, F, D), bf16),
                pltpu.VMEM((F, D), bf16),
                pltpu.VMEM((NG, T // 2, 128), i32),
                pltpu.VMEM((NG, (W + S) // 2, 128), i32),
                pltpu.VMEM((2 + S // 128, D // 2, 128), i32),
                pltpu.VMEM((NQ, D, 128), f32),
                pltpu.VMEM((3, 4, 256, 128), f32),
                pltpu.VMEM((T, D), f32),
                pltpu.VMEM((T // 2, D), i32),
                pltpu.SemaphoreType.DMA((7,)),
            ],
            compiler_params=pltpu.CompilerParams(dimension_semantics=("arbitrary",),
                                                 vmem_limit_bytes=100 * 1024 * 1024),
        )(x, A_wqkv, A_wo, B_w1.T, B_w3.T, B_w2)
        return out.reshape(1, S, D)
    return f


_impl = make()


@jax.jit
def pallas_sequential_preLN__sliding_block__glu_gated_swiglu__prompt_kernel(
    A_x: jax.Array,
    A_wqkv: jax.Array,
    A_wo: jax.Array,
    B_x: jax.Array,
    B_w1: jax.Array,
    B_w3: jax.Array,
    B_w2: jax.Array,
):
    return _impl(A_x, A_wqkv, A_wo, B_x, B_w1, B_w3, B_w2)
```

```python
import jax
import jax.numpy as jnp
import jax.experimental.pallas as pl
import jax.experimental.pallas.tpu as pltpu

S, D, F = 2048, 640, 1728
H, DH, W = 32, 20, 256
NG = 8
LOG2E = 1.4426950408889634
NEG = float('-inf')
f32 = jnp.float32
bf16 = jnp.bfloat16
i32 = jnp.int32
NT = (((1,), (1,)), ((), ()))
ONES_PK = 0x3F803F80
T = 256
NB = S // T


def _ln(x):
    m = jnp.mean(x, axis=-1, keepdims=True)
    xc = x - m
    v = jnp.mean(xc * xc, axis=-1, keepdims=True)
    return xc * jax.lax.rsqrt(v + 1e-5)


def _group_tile(a, g):
    lo = 80 * g
    t0, off = lo // 128, lo % 128
    ta = a[t0]
    if off + 80 <= 128:
        return ta
    tb = a[t0 + 1]
    lane = jax.lax.broadcasted_iota(i32, ta.shape, 1)
    return jnp.where(lane >= off, ta, tb)


def _swiglu(g, u):
    hg = 0.5 * g
    p = hg * u
    return p + p * jnp.tanh(hg)


def make(PAT0="qabcABC", DEP0=2, PAT="qaF4bAF4cBF4C", PATS="qaF4bAF4cBC", NSHORT=4, NPRE=10, NMID=0, NPOST=8,
         SEG=(4, 8), NOBC=0, VSPLIT=2, ONLY=None, DEP=1, PATL=None, DS=1, PACE=1, PACE0=0, TOK=(0, 64, 128, 192)):

    def attn_fns(first, tok, q_ref, k_ref, vt_ref, ot_ref, s_ref, p_ref, tokens):
        lane16 = jax.lax.broadcasted_iota(i32, (16, 128), 1)
        row16 = jax.lax.broadcasted_iota(i32, (16, 128), 0)
        lane32 = jax.lax.broadcasted_iota(i32, (32, 128), 1)
        row32 = jax.lax.broadcasted_iota(i32, (32, 128), 0)
        tri = row32 <= (lane32 % 32)
        b0 = (lane16 & 32) == 0
        b1 = (lane16 & 64) == 0
        b0_24 = (jax.lax.broadcasted_iota(i32, (24, 128), 1) & 32) == 0
        zero16 = jnp.zeros((16, 128), i32)
        pi_ref = p_ref.bitcast(i32)
        zs = pl.program_id(0) // 64
        dz = pl.multiple_of(zs * 8, 8)
        pace = PACE0 if first else PACE

        def sld(slot, j, r0):
            if DS == 1:
                return s_ref[slot][pl.ds(dz + 256 * j + r0, 32), :]
            return s_ref[slot][256 * j + r0:256 * j + r0 + 32, :]

        def info(qb):
            return max(8 - 4 * qb, 0) if first else 0

        def qk(slot, qb, g):
            miss = info(qb)
            masks = []
            for h in range(4):
                lo = (80 * g + 20 * h) % 128
                if lo + 20 <= 128:
                    msk = (lane16 >= lo) & (lane16 < lo + 20)
                else:
                    msk = (lane16 >= lo) | (lane16 < lo + 20 - 128)
                masks.append(jnp.where(msk, -1, 0))
            mxs = []
            for j in range(4):
                q = q_ref[g, qb * 64 + 16 * j: qb * 64 + 16 * j + 16, :]
                wq = pltpu.bitcast(jnp.concatenate([q & masks[m ^ j] for m in range(4)], axis=0), bf16)
                c0 = max(j, miss)
                c1 = j + 9
                nrows = (c1 - c0) * 32
                if first:
                    r0 = qb * 64 + 16 * c0
                    kk = k_ref[g, r0: r0 + nrows // 2, :]
                else:
                    kk = k_ref[g, pl.ds(pl.multiple_of(tok // 2 + qb * 64 + 16 * c0, 16), nrows // 2), :]
                s = jax.lax.dot_general(pltpu.bitcast(kk, bf16), wq, NT, preferred_element_type=f32)
                if j == 3:
                    tokens[:] = [s[(r * nrows // 256) // 8 * 8:(r * nrows // 256) // 8 * 8 + 8] for r in TOK]
                bot = s[nrows - 32:, :]
                if c0 == j:
                    sm = jnp.where(tri, bot, s[:32, :])
                    mid = s[32:nrows - 32, :]
                else:
                    sm = jnp.where(tri, bot, NEG)
                    mid = s[:nrows - 32, :] if nrows > 32 else None
                allm = sm if mid is None else jnp.concatenate([mid, sm], axis=0)
                n = allm.shape[0]
                s_ref[slot][256 * j + 256 - n:256 * j + 256, :] = allm
                parts = [allm[8 * t:8 * t + 8] for t in range(n // 8)]
                accs = parts[:4]
                for t in range(4, len(parts)):
                    accs[t % 4] = jnp.maximum(accs[t % 4], parts[t])
                m8 = jnp.maximum(jnp.maximum(accs[0], accs[1]), jnp.maximum(accs[2], accs[3]))
                mx = jnp.max(m8, axis=0, keepdims=True)
                mxs.append(jnp.broadcast_to(mx, (8, 128)))
            return dict(slot=slot, qb=qb, g=g, mxs=mxs, R=[None] * 4, pm={}, Z={})

        def exp_tile(st, t):
            slot, qb, g, mxs = st['slot'], st['qb'], st['g'], st['mxs']
            if 4 * t < info(qb):
                return
            Z = [[] for _ in range(4)]
            for c in range(4 * t, 4 * t + 4):
                if pace and tokens:
                    zero = pltpu.bitcast(pltpu.bitcast(tokens[(c % 4) * len(tokens) // 4], i32) & zs, f32)
                else:
                    zero = None

                def ex(j, r0):
                    m = mxs[j] if zero is None else mxs[j] + zero
                    return jnp.exp2(sld(slot, j, r0) - jnp.concatenate([m] * 4, axis=0))

                def pk(j):
                    if c < j or c > j + 8:
                        return None
                    if c == j or c == j + 8:
                        if j not in st['pm']:
                            st['pm'][j] = ex(j, 224)
                        pm = st['pm'][j]
                        v = jnp.where(tri, 0.0, pm) if c == j else jnp.where(tri, pm, 0.0)
                    else:
                        v = ex(j, 32 * (c - j - 1))
                    p_ref[32 * j:32 * j + 32, :] = v.astype(bf16)
                    return pi_ref[16 * j:16 * j + 16, :]

                def sel(mask, a, b):
                    if a is None and b is None:
                        return None
                    return jnp.where(mask, zero16 if a is None else a, zero16 if b is None else b)
                X = [pk(j) for j in range(4)]
                Y = [[sel(b0, X[2 * j1], X[2 * j1 + 1]), sel(b0, X[2 * j1 + 1], X[2 * j1])] for j1 in range(2)]
                for h0 in range(2):
                    Z[h0].append(sel(b1, Y[0][h0], Y[1][h0]))
                    Z[2 + h0].append(sel(b1, Y[1][h0], Y[0][h0]))
            st['Z'][t] = Z

        def mm_tiles(st, tl):
            qb, g = st['qb'], st['g']
            last = 2 in tl
            tl = [u for u in tl if u in st['Z']]
            if tl:
                for h in range(4):
                    hh = 4 * g + h
                    w0 = (20 * hh) // 16 * 16
                    o = 20 * hh - w0
                    vs = []
                    for u in tl:
                        if first:
                            v = vt_ref[qb + u, w0 // 2:w0 // 2 + 16, :]
                        else:
                            v = vt_ref[tok // 128 + qb + u, w0 // 2:w0 // 2 + 16, :]
                        ones_rows = (row16 >= 12) if o < 8 else (row16 < 4)
                        vs.append(jnp.where(ones_rows, ONES_PK, v))
                    v = pltpu.bitcast(jnp.concatenate(vs, axis=1) if len(vs) > 1 else vs[0], bf16)
                    ph = pltpu.bitcast(jnp.concatenate(sum([st['Z'][u][h] for u in tl], []), axis=0), bf16)
                    r = jnp.dot(v, ph, preferred_element_type=f32)
                    st['R'][h] = r if st['R'][h] is None else st['R'][h] + r
            if last:
                outs = []
                for h in range(4):
                    o = (20 * h) % 16
                    r = st['R'][h]
                    if o < 8:
                        l8, dat = r[24:32, :], r[0:24, :]
                    else:
                        l8, dat = r[0:8, :], r[8:32, :]
                    inv = pl.reciprocal(l8, approx=True)
                    inv = inv * (2.0 - l8 * inv)
                    dat = dat * jnp.concatenate([inv, inv, inv], axis=0)
                    if h == 1:
                        dat = jnp.where(b0_24, pltpu.roll(dat, 96, 1), pltpu.roll(dat, 32, 1))
                    elif h == 2:
                        dat = pltpu.roll(dat, 64, 1)
                    elif h == 3:
                        dat = jnp.where(b0_24, pltpu.roll(dat, 32, 1), pltpu.roll(dat, 96, 1))
                    outs.append(dat)
                sub = jax.lax.broadcasted_iota(i32, (8, 128), 0)
                og = jnp.concatenate([
                    outs[0][0:16], jnp.where(sub < 4, outs[0][16:24], outs[1][0:8]), outs[1][8:24],
                    outs[2][0:16], jnp.where(sub < 4, outs[2][16:24], outs[3][0:8]), outs[3][8:24]], axis=0)
                ot_ref[qb, 80 * g:80 * g + 80, :] = og
        return qk, exp_tile, mm_tiles

    def kern(x_hbm, wqkv_hbm, wo_hbm, w1t_hbm, w3t_hbm, w2_hbm, o_ref,
             x_ref, wqkv_ref, wvt_ref, wo_ref, w13_ref, w2_ref, q0, q1, k_ref, vt_ref, ot0, ot1, s0, s1, s2,
             h_ref, hn_ref, p0, p1, sems):
        s_ref = [s0, s1, s2]
        s_id = pl.program_id(0)

        def xcopy(b):
            return pltpu.make_async_copy(x_hbm.at[b], x_ref.at[b], sems.at[7 + b])

        def wcol(a, b, k):
            return pltpu.make_async_copy(wqkv_hbm.at[:, a:b], wqkv_ref.at[:, a:b], sems.at[k])

        class FFN:
            def __init__(self, slot_old, slot_hn, tokens):
                self.slot_old, self.slot_hn, self.tokens = slot_old, slot_hn, tokens
                self.jobs = [('up', n) for n in range(27)] + [('down', n) for n in range(5)]
                self.k = 0
                self.acc = None
                self.gate = None
                self.acts = []
                self.left = 27 * 5 + 5 * 14

            def emit(self, npass):
                npass = min(npass, self.left)
                self.left -= npass
                while npass > 0:
                    kind, n = self.jobs[0]
                    kt = 5 if kind == 'up' else 14
                    m = min(npass, kt - self.k)
                    k0, k1 = self.k, self.k + m
                    if kind == 'up':
                        lhs = pltpu.bitcast(hn_ref[self.slot_hn, :, 128 * k0:128 * k1], bf16)
                        if n < 26:
                            c = n // 2
                            w = w13_ref[n % 2, 128 * c:128 * c + 128, 128 * k0:128 * k1]
                        else:
                            w = jnp.concatenate([w13_ref[0, 1664:1728, 128 * k0:128 * k1],
                                                 w13_ref[1, 1664:1728, 128 * k0:128 * k1]], axis=0)
                        r = jax.lax.dot_general(lhs, w, NT, preferred_element_type=f32)
                    else:
                        r = None
                        for c in range(k0, k1):
                            kw = 128 if c < 13 else 64
                            rr = jnp.dot(self.acts[c], w2_ref[128 * c:128 * c + kw, 128 * n:128 * n + 128],
                                         preferred_element_type=f32)
                            r = rr if r is None else r + rr
                    self.acc = r if self.acc is None else self.acc + r
                    self.tokens[:] = [self.acc[r0:r0 + 8] for r0 in TOK]
                    self.k = k1
                    npass -= m
                    if self.k == kt:
                        if kind == 'down':
                            o_ref[:, 128 * n:128 * n + 128] = (
                                h_ref[self.slot_old, :, 128 * n:128 * n + 128] + self.acc).astype(bf16)
                        elif n == 26:
                            a = _swiglu(self.acc, pltpu.roll(self.acc, 64, 1))
                            self.acts.append(a[:, :64].astype(bf16))
                        elif n % 2 == 0:
                            self.gate = self.acc
                        else:
                            self.acts.append(_swiglu(self.gate, self.acc).astype(bf16))
                        self.acc = None
                        self.k = 0
                        self.jobs.pop(0)

        def qk_tiles(xn, a, b):
            r = jnp.dot(xn, wqkv_ref[:, 128 * a:128 * b], preferred_element_type=f32)
            out = []
            for t in range(a, b):
                v = r[:, 128 * (t - a):128 * (t - a + 1)]
                if t < 5:
                    v = v * (DH ** -0.5 * LOG2E)
                out.append(pltpu.bitcast(v.astype(bf16), i32))
            return out

        def store_qk(first, tiles, tok):
            q_ref = q0 if first else q1
            for g in range(NG):
                q_ref[g] = _group_tile(tiles[:5], g)
            for g in range(NG):
                kg = _group_tile(tiles[5:], g)
                if first:
                    k_ref[g, W // 2:W // 2 + T, :] = kg
                else:
                    k_ref[g, pl.ds(pl.multiple_of(W // 2 + tok // 2, T // 2), T // 2), :] = kg

        def store_vt(first, nrows, xnv, tok, nsplit):
            rs = D // nsplit
            for u in range(nsplit):
                vt = jax.lax.dot_general(wvt_ref[rs * u:rs * u + rs, :], xnv, NT, preferred_element_type=f32).astype(bf16)
                vt = pltpu.bitcast(vt, i32)
                for t in range(nrows // 128):
                    if first:
                        vt_ref[2 + t, rs * u // 2:(rs * u + rs) // 2, :] = vt[:, t * 128:(t + 1) * 128]
                    else:
                        vt_ref[2 + tok // 128 + t, rs * u // 2:(rs * u + rs) // 2, :] = vt[:, t * 128:(t + 1) * 128]

        def run_attn(first, nq, tok, dep, pats, ffn, tokens):
            qk, exp_tile, mm_tiles = attn_fns(first, tok, q0 if first else q1, k_ref, vt_ref,
                                              ot0 if first else ot1, s_ref, p0 if first else p1, tokens)
            items = [(qb, g) for qb in range(nq) for g in range(NG)]
            n = len(items)
            NS = dep + 1
            ss = {}
            for t in range(min(dep, n)):
                ss[t] = qk(t % NS, *items[t])
            if ffn is not None:
                ffn.emit(NMID)
            for t in range(n + 1):
                pat = pats[min(t, n - 1)]
                p = 0
                while p < len(pat):
                    ch = pat[p]
                    if ch == 'F':
                        e = p + 1
                        while e < len(pat) and pat[e].isdigit():
                            e += 1
                        if t < n:
                            ffn.emit(int(pat[p + 1:e]))
                        p = e - 1
                    elif ch in 'xyzw':
                        if t > 0:
                            mm_tiles(ss[t - 1], [0, 1, 2] if ch == 'w' else ['xyz'.index(ch)])
                    elif t == n:
                        pass
                    elif ch == 'q':
                        if t + dep < n:
                            ss[t + dep] = qk((t + dep) % NS, *items[t + dep])
                    elif ch in 'abc':
                        exp_tile(ss[t], 'abc'.index(ch))
                    elif ch in 'ABC':
                        mm_tiles(ss[t], ['ABC'.index(ch)])
                    elif ch == 'W':
                        mm_tiles(ss[t], [0, 1, 2])
                    p += 1
                if t == n - 1 and ffn is not None and any(ch in pat for ch in 'xyzw'):
                    ffn.emit(4)

        def wo_proj(x, ot_ref, qbs):
            o = [ot_ref[qb].T for qb in qbs]
            o = (jnp.concatenate(o, axis=0) if len(o) > 1 else o[0]).astype(bf16)
            return x + jnp.dot(o, wo_ref[...], preferred_element_type=f32)

        @pl.when(s_id == 0)
        def _():
            if ONLY == 'mid':
                return
            s1, s2 = SEG
            cx = [xcopy(0), xcopy(1), xcopy(2)]
            ca = wcol(0, 128 * s1, 0)
            cb = wcol(128 * s1, 128 * s2, 1)
            cc = wcol(128 * s2, 3 * D, 2)
            cw = [pltpu.make_async_copy(wo_hbm, wo_ref, sems.at[3]),
                  pltpu.make_async_copy(w1t_hbm, w13_ref.at[0], sems.at[4]),
                  pltpu.make_async_copy(w3t_hbm, w13_ref.at[1], sems.at[5]),
                  pltpu.make_async_copy(w2_hbm, w2_ref, sems.at[6])]
            for c in [cx[0], cx[1], ca, cb, cc, cw[0], cx[2]] + cw[1:]:
                c.start()
            cx[0].wait()
            xn0 = _ln(x_ref[0].astype(f32))
            cx[1].wait()
            xn1 = _ln(x_ref[1].astype(f32))
            xn = jnp.concatenate([xn0, xn1], axis=0).astype(bf16)
            ca.wait()
            tiles = qk_tiles(xn, 0, s1)
            cb.wait()
            tiles += qk_tiles(xn, s1, s2)
            cc.wait()
            cw[0].wait()
            wvt_ref[...] = wqkv_ref[:, 2 * D:].astype(f32).T.astype(bf16)
            tiles += qk_tiles(xn, s2, 10)
            store_qk(True, tiles, 0)
            store_vt(True, 2 * T, xn, 0, 1)
            run_attn(True, 4, 0, DEP0, [PAT0] * 32, None, [])
            for qb in range(4):
                blk, half = qb // 2, qb % 2
                h = wo_proj(x_ref[blk, 128 * half:128 * half + 128, :].astype(f32), ot0, [qb])
                h_ref[blk, 128 * half:128 * half + 128, :] = h
                hn_ref[blk, 64 * half:64 * half + 64, :] = pltpu.bitcast(_ln(h).astype(bf16), i32)
            for c in cw[1:]:
                c.wait()

        slot_old = (s_id + 2) % 3
        slot_new = (s_id + 1) % 3
        slot_hn = (s_id + 1) % 2

        @pl.when((s_id > 0) & (s_id < NB - 2))
        def _():
            xcopy(s_id + 2).start()

        @pl.when((s_id > 0) & (s_id < NB - 1))
        def _():
            xcopy(s_id + 1).wait()
            if ONLY == 'pro':
                return
            tokens = []
            ffn = FFN(slot_old, slot_hn, tokens)
            ffn.emit(NPRE)
            xn = _ln(x_ref[s_id + 1].astype(f32)).astype(bf16)
            tok = pl.multiple_of((s_id + 1) * T, T)
            store_qk(False, qk_tiles(xn, 0, 10), tok)
            store_vt(False, T, xn, tok, VSPLIT)
            pats = [PATS if (t * NSHORT) % 16 < NSHORT else PAT for t in range(16)]
            if PATL is not None:
                pats = PATL
            run_attn(False, 2, tok, DEP, pats, ffn, tokens)
            ffn.emit(NPOST)
            h = wo_proj(x_ref[s_id + 1].astype(f32), ot1, [0, 1])
            h_ref[slot_new] = h
            assert ffn.left <= 70, ffn.left
            hn_ref[slot_hn] = pltpu.bitcast(_ln(h).astype(bf16), i32)
            ffn.emit(1000)

        @pl.when(s_id >= NB - 1)
        def _():
            if ONLY is None:
                FFN(slot_old, slot_hn, []).emit(1000)

    @jax.jit
    def f(A_x, A_wqkv, A_wo, B_x, B_w1, B_w3, B_w2):
        x = A_x.reshape(NB, T, D)
        anyspec = pl.BlockSpec(memory_space=pl.ANY)
        out = pl.pallas_call(
            kern,
            out_shape=jax.ShapeDtypeStruct((S, D), bf16),
            grid=(NB + 1,),
            in_specs=[anyspec] * 6,
            out_specs=pl.BlockSpec((T, D), lambda i: (jnp.maximum(i - 1, 0), 0)),
            scratch_shapes=[
                pltpu.VMEM((NB, T, D), bf16),
                pltpu.VMEM((D, 3 * D), bf16),
                pltpu.VMEM((D, D), bf16),
                pltpu.VMEM((D, D), bf16),
                pltpu.VMEM((2, F, D), bf16),
                pltpu.VMEM((F, D), bf16),
                pltpu.VMEM((NG, T, 128), i32),
                pltpu.VMEM((NG, T // 2, 128), i32),
                pltpu.VMEM((NG, (W + S) // 2, 128), i32),
                pltpu.VMEM((2 + S // 128, D // 2, 128), i32),
                pltpu.VMEM((4, D, 128), f32),
                pltpu.VMEM((2, D, 128), f32),
                pltpu.VMEM((1024, 128), f32),
                pltpu.VMEM((1024, 128), f32),
                pltpu.VMEM((1024, 128), f32),
                pltpu.VMEM((3, T, D), f32),
                pltpu.VMEM((2, T // 2, D), i32),
                pltpu.VMEM((128, 128), bf16),
                pltpu.VMEM((128, 128), bf16),
                pltpu.SemaphoreType.DMA((7 + NB,)),
            ],
            compiler_params=pltpu.CompilerParams(dimension_semantics=("arbitrary",),
                                                 vmem_limit_bytes=100 * 1024 * 1024,
                                                 disable_bounds_checks=bool(NOBC)),
        )(x, A_wqkv, A_wo, B_w1.T, B_w3.T, B_w2)
        return out.reshape(1, S, D)
    return f


_impl = make(NSHORT=16,PATS='qaF4wbF4c')


@jax.jit
def pallas_sequential_preLN__sliding_block__glu_gated_swiglu__prompt_kernel(
    A_x: jax.Array,
    A_wqkv: jax.Array,
    A_wo: jax.Array,
    B_x: jax.Array,
    B_w1: jax.Array,
    B_w3: jax.Array,
    B_w2: jax.Array,
):
    return _impl(A_x, A_wqkv, A_wo, B_x, B_w1, B_w3, B_w2)
```

```python
import jax
import jax.numpy as jnp
import jax.experimental.pallas as pl
import jax.experimental.pallas.tpu as pltpu

S, D, F = 2048, 640, 1728
H, DH, W = 32, 20, 256
NG = 8
LOG2E = 1.4426950408889634
f32 = jnp.float32
bf16 = jnp.bfloat16
i32 = jnp.int32
NT = (((1,), (1,)), ((), ()))
ONES_PK = 0x3F803F80
T = 256
NB = S // T


def _ln(x):
    m = jnp.mean(x, axis=-1, keepdims=True)
    xc = x - m
    v = jnp.mean(xc * xc, axis=-1, keepdims=True)
    return xc * jax.lax.rsqrt(v + 1e-5)


def _group_tile(a, g):
    lo = 80 * g
    t0, off = lo // 128, lo % 128
    ta = a[t0]
    if off + 80 <= 128:
        return ta
    lane = jax.lax.broadcasted_iota(i32, ta.shape, 1)
    return jnp.where(lane >= off, ta, a[t0 + 1])


def _swiglu(g, u):
    hg = 0.5 * g
    p = hg * u
    return p + p * jnp.tanh(hg)


def make(PAT0="qabcABC", PATF="qJabcABC", DEP0=2, PAT="qaF4wbF4c", NPRE=10, NPOST=8, NOBC=1,
         TOK=(32, 96, 160, 224), FILL0=(0, 1, 3, 5, 7, 9), ONLY=None):

    def attn_fns(first, blk, q_ref, k_ref, vt_ref, ot_ref, s_ref, p_ref, tokens):
        lane16 = jax.lax.broadcasted_iota(i32, (16, 128), 1)
        row16 = jax.lax.broadcasted_iota(i32, (16, 128), 0)
        lane32 = jax.lax.broadcasted_iota(i32, (32, 128), 1)
        row32 = jax.lax.broadcasted_iota(i32, (32, 128), 0)
        tri = row32 <= (lane32 % 32)
        b0 = (lane16 & 32) == 0
        b1 = (lane16 & 64) == 0
        b0_24 = (jax.lax.broadcasted_iota(i32, (24, 128), 1) & 32) == 0
        zero16 = jnp.zeros((16, 128), i32)
        pi_ref = p_ref.bitcast(i32)
        zs = jax.lax.shift_right_logical(pl.program_id(0), 6)
        dz = pl.multiple_of(zs * 8, 8)

        def miss_of(qb):
            return max(8 - 4 * qb, 0) if first else 0

        def qk(slot, qb, g):
            miss = miss_of(qb)
            masks = []
            for h in range(4):
                lo = (80 * g + 20 * h) % 128
                if lo + 20 <= 128:
                    msk = (lane16 >= lo) & (lane16 < lo + 20)
                else:
                    msk = (lane16 >= lo) | (lane16 < lo + 20 - 128)
                masks.append(jnp.where(msk, -1, 0))
            mxs = []
            for j in range(4):
                q = q_ref[g, qb * 64 + 16 * j: qb * 64 + 16 * j + 16, :]
                wq = pltpu.bitcast(jnp.concatenate([q & masks[m ^ j] for m in range(4)], axis=0), bf16)
                c0 = max(j, miss)
                nrows = (j + 9 - c0) * 32
                if first:
                    r0 = qb * 64 + 16 * c0
                    kk = k_ref[g, r0: r0 + nrows // 2, :]
                else:
                    kk = k_ref[g, pl.ds(pl.multiple_of(blk * (T // 2) + qb * 64 + 16 * c0, 16), nrows // 2), :]
                s = jax.lax.dot_general(pltpu.bitcast(kk, bf16), wq, NT, preferred_element_type=f32)
                if j == 3:
                    tokens[:] = [s[(r * nrows // 256) // 8 * 8:(r * nrows // 256) // 8 * 8 + 8] for r in TOK]
                bot = s[nrows - 32:, :]
                if c0 == j:
                    sm = jnp.where(tri, bot, s[:32, :])
                    mid = s[32:nrows - 32, :]
                else:
                    sm = jnp.where(tri, bot, float('-inf'))
                    mid = s[:nrows - 32, :] if nrows > 32 else None
                allm = sm if mid is None else jnp.concatenate([mid, sm], axis=0)
                n = allm.shape[0]
                s_ref[slot][256 * j + 256 - n:256 * j + 256, :] = allm
                parts = [allm[8 * t:8 * t + 8] for t in range(n // 8)]
                accs = parts[:4]
                for t in range(4, len(parts)):
                    accs[t % 4] = jnp.maximum(accs[t % 4], parts[t])
                m8 = jnp.maximum(jnp.maximum(accs[0], accs[1]), jnp.maximum(accs[2], accs[3]))
                mx = jnp.max(m8, axis=0, keepdims=True)
                mxs.append(jnp.broadcast_to(mx, (8, 128)))
            return dict(slot=slot, qb=qb, g=g, mxs=mxs, R=[None] * 4, pm={}, Z={})

        def exp_tile(st, t):
            slot, qb, mxs = st['slot'], st['qb'], st['mxs']
            if 4 * t < miss_of(qb):
                return
            Z = [[] for _ in range(4)]
            for c in range(4 * t, 4 * t + 4):
                zero = None if first else pltpu.bitcast(pltpu.bitcast(tokens[c % 4], i32) & zs, f32)

                def ex(j, r0):
                    m = mxs[j] if zero is None else mxs[j] + zero
                    sv = s_ref[slot][pl.ds(dz + 256 * j + r0, 32), :]
                    return jnp.exp2(sv - jnp.concatenate([m] * 4, axis=0))

                def pk(j):
                    if c < j or c > j + 8:
                        return None
                    if c == j or c == j + 8:
                        if j not in st['pm']:
                            st['pm'][j] = ex(j, 224)
                        pm = st['pm'][j]
                        v = jnp.where(tri, 0.0, pm) if c == j else jnp.where(tri, pm, 0.0)
                    else:
                        v = ex(j, 32 * (c - j - 1))
                    p_ref[32 * j:32 * j + 32, :] = v.astype(bf16)
                    return pi_ref[16 * j:16 * j + 16, :]

                def sel(mask, a, b):
                    if a is None and b is None:
                        return None
                    return jnp.where(mask, zero16 if a is None else a, zero16 if b is None else b)
                X = [pk(j) for j in range(4)]
                Y = [[sel(b0, X[2 * j1], X[2 * j1 + 1]), sel(b0, X[2 * j1 + 1], X[2 * j1])] for j1 in range(2)]
                for h0 in range(2):
                    Z[h0].append(sel(b1, Y[0][h0], Y[1][h0]))
                    Z[2 + h0].append(sel(b1, Y[1][h0], Y[0][h0]))
            st['Z'][t] = Z

        def mm_tiles(st, tl):
            qb, g = st['qb'], st['g']
            last = 2 in tl
            tl = [u for u in tl if u in st['Z']]
            if tl:
                for h in range(4):
                    hh = 4 * g + h
                    w0 = (20 * hh) // 16 * 16
                    o = 20 * hh - w0
                    vs = []
                    for u in tl:
                        v = vt_ref[blk * 2 + qb + u, w0 // 2:w0 // 2 + 16, :]
                        ones_rows = (row16 >= 12) if o < 8 else (row16 < 4)
                        vs.append(jnp.where(ones_rows, ONES_PK, v))
                    v = pltpu.bitcast(jnp.concatenate(vs, axis=1) if len(vs) > 1 else vs[0], bf16)
                    ph = pltpu.bitcast(jnp.concatenate(sum([st['Z'][u][h] for u in tl], []), axis=0), bf16)
                    r = jnp.dot(v, ph, preferred_element_type=f32)
                    st['R'][h] = r if st['R'][h] is None else st['R'][h] + r
            if last:
                outs = []
                for h in range(4):
                    o = (20 * h) % 16
                    r = st['R'][h]
                    if o < 8:
                        l8, dat = r[24:32, :], r[0:24, :]
                    else:
                        l8, dat = r[0:8, :], r[8:32, :]
                    inv = pl.reciprocal(l8, approx=True)
                    inv = inv * (2.0 - l8 * inv)
                    dat = dat * jnp.concatenate([inv, inv, inv], axis=0)
                    if h == 1:
                        dat = jnp.where(b0_24, pltpu.roll(dat, 96, 1), pltpu.roll(dat, 32, 1))
                    elif h == 2:
                        dat = pltpu.roll(dat, 64, 1)
                    elif h == 3:
                        dat = jnp.where(b0_24, pltpu.roll(dat, 32, 1), pltpu.roll(dat, 96, 1))
                    outs.append(dat)
                sub = jax.lax.broadcasted_iota(i32, (8, 128), 0)
                og = jnp.concatenate([
                    outs[0][0:16], jnp.where(sub < 4, outs[0][16:24], outs[1][0:8]), outs[1][8:24],
                    outs[2][0:16], jnp.where(sub < 4, outs[2][16:24], outs[3][0:8]), outs[3][8:24]], axis=0)
                ot_ref[qb, 80 * g:80 * g + 80, :] = og
        return qk, exp_tile, mm_tiles

    def kern(x_hbm, wqkv_hbm, wo_hbm, w1t_hbm, w3t_hbm, w2_hbm, o_hbm,
             x_ref, wqkv_ref, wvt_ref, wo_ref, w13_ref, w2_ref, q0, q1, k_ref, vt_ref, ot0, ot1,
             s0, s1, s2, h_ref, hn_ref, p0, p1, o_ref, sems, osem):
        s_ref = [s0, s1, s2]
        s_id = pl.program_id(0)

        def xrest():
            return pltpu.make_async_copy(x_hbm.at[3:NB], x_ref.at[3:NB], sems.at[7])

        class FFN:
            def __init__(self, tokens):
                self.tokens = tokens
                self.blk = s_id - 1
                self.jobs = [('up', n) for n in range(27)] + [('down', n) for n in range(5)]
                self.k = 0
                self.acc = None
                self.gate = None
                self.acts = []
                self.left = 27 * 5 + 5 * 14

            def emit(self, npass):
                npass = min(npass, self.left)
                self.left -= npass
                while npass > 0:
                    kind, n = self.jobs[0]
                    kt = 5 if kind == 'up' else 14
                    m = min(npass, kt - self.k)
                    k0, k1 = self.k, self.k + m
                    if kind == 'up':
                        lhs = pltpu.bitcast(hn_ref[self.blk & 1, :, 128 * k0:128 * k1], bf16)
                        if n < 26:
                            c = n // 2
                            w = w13_ref[n % 2, 128 * c:128 * c + 128, 128 * k0:128 * k1]
                        else:
                            w = jnp.concatenate([w13_ref[0, 1664:1728, 128 * k0:128 * k1],
                                                 w13_ref[1, 1664:1728, 128 * k0:128 * k1]], axis=0)
                        r = jax.lax.dot_general(lhs, w, NT, preferred_element_type=f32)
                    else:
                        r = None
                        for c in range(k0, k1):
                            kw = 128 if c < 13 else 64
                            rr = jnp.dot(self.acts[c], w2_ref[128 * c:128 * c + kw, 128 * n:128 * n + 128],
                                         preferred_element_type=f32)
                            r = rr if r is None else r + rr
                    self.acc = r if self.acc is None else self.acc + r
                    self.tokens[:] = [self.acc[r0:r0 + 8] for r0 in TOK]
                    self.k = k1
                    npass -= m
                    if self.k == kt:
                        if kind == 'down':
                            o_ref[self.blk, n] = (h_ref[self.blk & 3, :, 128 * n:128 * n + 128] + self.acc).astype(bf16)
                            pltpu.make_async_copy(o_ref.at[self.blk, n],
                                                  o_hbm.at[self.blk, :, 128 * n:128 * n + 128], osem.at[0]).start()
                        elif n == 26:
                            a = _swiglu(self.acc, pltpu.roll(self.acc, 64, 1))
                            self.acts.append(a[:, :64].astype(bf16))
                        elif n % 2 == 0:
                            self.gate = self.acc
                        else:
                            self.acts.append(_swiglu(self.gate, self.acc).astype(bf16))
                        self.acc = None
                        self.k = 0
                        self.jobs.pop(0)

        def qk_tiles(xn, a, b):
            r = jnp.dot(xn, wqkv_ref[:, 128 * a:128 * b], preferred_element_type=f32)
            out = []
            for t in range(a, b):
                v = r[:, 128 * (t - a):128 * (t - a + 1)]
                if t < 5:
                    v = v * (DH ** -0.5 * LOG2E)
                out.append(pltpu.bitcast(v.astype(bf16), i32))
            return out

        def store_qk(first, tiles, blk):
            hT = T // 2
            for g in range(NG):
                if first:
                    q0[g, blk * hT:blk * hT + hT, :] = _group_tile(tiles[:5], g)
                else:
                    q1[g] = _group_tile(tiles[:5], g)
            for g in range(NG):
                kg = _group_tile(tiles[5:], g)
                if first:
                    k_ref[g, W // 2 + blk * hT:W // 2 + blk * hT + hT, :] = kg
                else:
                    k_ref[g, pl.ds(pl.multiple_of(W // 2 + blk * hT, hT), hT), :] = kg

        def store_vt(xn, blk):
            for u in range(2):
                vt = jax.lax.dot_general(wvt_ref[320 * u:320 * u + 320, :], xn, NT, preferred_element_type=f32)
                vt = pltpu.bitcast(vt.astype(bf16), i32)
                for t in range(2):
                    vt_ref[2 + blk * 2 + t, 160 * u:160 * u + 160, :] = vt[:, t * 128:(t + 1) * 128]

        def run_attn(first, nq, blk, dep, pats, filler, tokens):
            qk, exp_tile, mm_tiles = attn_fns(first, blk, q0 if first else q1, k_ref, vt_ref,
                                              ot0 if first else ot1, s_ref, p0 if first else p1, tokens)
            items = [(qb, g) for qb in range(nq) for g in range(NG)]
            n = len(items)
            ss = {}
            for t in range(dep):
                ss[t] = qk(t % (dep + 1), *items[t])
            for t in range(n + 1):
                pat = pats[min(t, n - 1)]
                for p, ch in enumerate(pat):
                    if ch == 'w':
                        if t > 0:
                            mm_tiles(ss[t - 1], [0, 1, 2])
                    elif t == n or ch.isdigit():
                        pass
                    elif ch == 'F':
                        filler.emit(int(pat[p + 1]))
                    elif ch == 'J':
                        filler(t)
                    elif ch == 'q':
                        if t + dep < n:
                            ss[t + dep] = qk((t + dep) % (dep + 1), *items[t + dep])
                    elif ch in 'abc':
                        exp_tile(ss[t], 'abc'.index(ch))
                    else:
                        mm_tiles(ss[t], ['ABC'.index(ch)])
                if t == n - 1 and 'w' in pat:
                    filler.emit(4)

        def wo_proj(x, ot_ref, qbs):
            o = [ot_ref[qb].T for qb in qbs]
            o = (jnp.concatenate(o, axis=0) if len(o) > 1 else o[0]).astype(bf16)
            return x + jnp.dot(o, wo_ref[...], preferred_element_type=f32)

        @pl.when(s_id == 0)
        def _():
            if ONLY == 'mid':
                return

            def hcopy(src, dst, k):
                return pltpu.make_async_copy(src, dst, sems.at[k])

            def wcol(a, b, k):
                return hcopy(wqkv_hbm.at[:, a:b], wqkv_ref.at[:, a:b], k)
            cx0, cx1 = hcopy(x_hbm.at[0], x_ref.at[0], 0), hcopy(x_hbm.at[1], x_ref.at[1], 1)
            ca = wcol(0, 256, 2)
            cb = wcol(256, 768, 3)
            cc = [wcol(2 * D, 3 * D, 4), wcol(768, 1024, 4)]
            cd = [wcol(1024, 1280, 5), hcopy(wo_hbm, wo_ref, 5)]
            ce = [hcopy(x_hbm.at[2], x_ref.at[2], 6), hcopy(w1t_hbm, w13_ref.at[0], 6),
                  hcopy(w3t_hbm, w13_ref.at[1], 6), hcopy(w2_hbm, w2_ref, 6)]
            for c in [cx0, cx1, ca, cb] + cc + cd + ce + [xrest()]:
                c.start()
            cx0.wait()
            xn0 = _ln(x_ref[0].astype(f32))
            cx1.wait()
            xn1 = _ln(x_ref[1].astype(f32))
            xn = jnp.concatenate([xn0, xn1], axis=0).astype(bf16)
            xh = [xn[:T], xn[T:]]
            tiles = [[], []]

            def split_tiles(a, b, blks=(0, 1)):
                for u in blks:
                    tiles[u] += qk_tiles(xh[u], a, b)
            ca.wait()
            split_tiles(0, 2)
            cb.wait()
            for tl in qk_tiles(xn, 2, 6):
                tiles[0].append(tl[:T // 2])
                tiles[1].append(tl[T // 2:])
            for c in cc:
                c.wait()
            wvt_ref[...] = wqkv_ref[:, 2 * D:].astype(f32).T.astype(bf16)
            split_tiles(6, 8)
            store_vt(xh[0], 0)

            def vjob(u, t):
                def run():
                    vt = jax.lax.dot_general(wvt_ref[320 * u:320 * u + 320, :], xh[1][128 * t:128 * t + 128], NT,
                                             preferred_element_type=f32)
                    vt_ref[4 + t, 160 * u:160 * u + 160, :] = pltpu.bitcast(vt.astype(bf16), i32)
                return run

            def kjob(t):
                def run():
                    split_tiles(t, t + 1, (1,))
                    if t == 9:
                        store_qk(True, tiles[1], 1)
                return run
            jobs = [kjob(8), kjob(9)] + [vjob(u, t) for t in range(2) for u in range(2)]
            for c in cd:
                c.wait()
            split_tiles(8, 10, (0,))
            store_qk(True, tiles[0], 0)
            run_attn(True, 4, 0, DEP0, [PATF if t in FILL0 else PAT0 for t in range(32)],
                     lambda t: jobs.pop(0)(), [])
            assert not jobs
            for qb in range(4):
                blk, half = qb // 2, qb % 2
                h = wo_proj(x_ref[blk, 128 * half:128 * half + 128, :].astype(f32), ot0, [qb])
                h_ref[blk, 128 * half:128 * half + 128, :] = h
                hn_ref[blk, 64 * half:64 * half + 64, :] = pltpu.bitcast(_ln(h).astype(bf16), i32)
            for c in ce:
                c.wait()

        @pl.when(s_id == 2)
        def _():
            xrest().wait()

        @pl.when((s_id > 0) & (s_id < NB - 1))
        def _():
            if ONLY == 'pro':
                return
            blk = s_id + 1
            tokens = []
            ffn = FFN(tokens)
            ffn.emit(NPRE)
            xn = _ln(x_ref[blk].astype(f32)).astype(bf16)
            store_qk(False, qk_tiles(xn, 0, 10), blk)
            store_vt(xn, blk)
            run_attn(False, 2, blk, 1, [PAT] * 16, ffn, tokens)
            ffn.emit(NPOST)
            h = wo_proj(x_ref[blk].astype(f32), ot1, [0, 1])
            h_ref[blk & 3] = h
            assert ffn.left <= 70
            hn_ref[blk & 1] = pltpu.bitcast(_ln(h).astype(bf16), i32)
            ffn.emit(1000)

        @pl.when(s_id >= NB - 1)
        def _():
            if ONLY != 'mid':
                FFN([]).emit(1000)

        @pl.when(s_id == NB)
        def _():
            pltpu.make_async_copy(o_ref, o_ref, osem.at[0]).wait()

    @jax.jit
    def f(A_x, A_wqkv, A_wo, B_x, B_w1, B_w3, B_w2):
        x = A_x.reshape(NB, T, D)
        anyspec = pl.BlockSpec(memory_space=pl.ANY)
        out = pl.pallas_call(
            kern,
            out_shape=jax.ShapeDtypeStruct((NB, T, D), bf16),
            grid=(NB + 1,),
            in_specs=[anyspec] * 6,
            out_specs=anyspec,
            scratch_shapes=[
                pltpu.VMEM((NB, T, D), bf16),
                pltpu.VMEM((D, 3 * D), bf16),
                pltpu.VMEM((D, D), bf16),
                pltpu.VMEM((D, D), bf16),
                pltpu.VMEM((2, F, D), bf16),
                pltpu.VMEM((F, D), bf16),
                pltpu.VMEM((NG, T, 128), i32),
                pltpu.VMEM((NG, T // 2, 128), i32),
                pltpu.VMEM((NG, (W + S) // 2, 128), i32),
                pltpu.VMEM((2 + S // 128, D // 2, 128), i32),
                pltpu.VMEM((4, D, 128), f32),
                pltpu.VMEM((2, D, 128), f32),
                pltpu.VMEM((1024, 128), f32),
                pltpu.VMEM((1024, 128), f32),
                pltpu.VMEM((1024, 128), f32),
                pltpu.VMEM((4, T, D), f32),
                pltpu.VMEM((2, T // 2, D), i32),
                pltpu.VMEM((128, 128), bf16),
                pltpu.VMEM((128, 128), bf16),
                pltpu.VMEM((NB, 5, T, 128), bf16),
                pltpu.SemaphoreType.DMA((8,)),
                pltpu.SemaphoreType.DMA((1,)),
            ],
            compiler_params=pltpu.CompilerParams(dimension_semantics=("arbitrary",),
                                                 vmem_limit_bytes=100 * 1024 * 1024,
                                                 disable_bounds_checks=bool(NOBC)),
        )(x, A_wqkv, A_wo, B_w1.T, B_w3.T, B_w2)
        return out.reshape(1, S, D)
    return f


_impl = make()


@jax.jit
def pallas_sequential_preLN__sliding_block__glu_gated_swiglu__prompt_kernel(
    A_x: jax.Array,
    A_wqkv: jax.Array,
    A_wo: jax.Array,
    B_x: jax.Array,
    B_w1: jax.Array,
    B_w3: jax.Array,
    B_w2: jax.Array,
):
    return _impl(A_x, A_wqkv, A_wo, B_x, B_w1, B_w3, B_w2)
```

```python
import jax
import jax.numpy as jnp
import jax.experimental.pallas as pl
import jax.experimental.pallas.tpu as pltpu

S, D, F = 2048, 640, 1728
H, DH, W = 32, 20, 256
NG = 8
T = 256
NB = S // T
LOG2E = 1.4426950408889634
f32 = jnp.float32
bf16 = jnp.bfloat16
i32 = jnp.int32
NT = (((1,), (1,)), ((), ()))
ONES_PK = 0x3F803F80

PAT_FIRST, PAT_FIRST_FILL, FILL_AT = "qabcABC", "qJabcABC", (0, 1, 3, 6, 9, 12)
PAT_MID = "qaF4wbF4c"
TOK = (32, 96, 160, 224)


def _ln(x, zeros=None):
    m = jnp.mean(x, axis=-1, keepdims=True)
    if zeros:
        rep = x.shape[0] // (8 * len(zeros))
        m = m + jnp.concatenate([z[:, :1] for z in zeros for _ in range(rep)], axis=0)
    mb = m.astype(bf16).astype(f32)
    xc = x - mb
    dm = m - mb
    v = jnp.mean(xc * xc, axis=-1, keepdims=True) - dm * dm
    return xc * jax.lax.rsqrt(v + 1e-5)


def _group_tile(a, g):
    lo = 80 * g
    t0, off = lo // 128, lo % 128
    ta = a[t0]
    if off + 80 <= 128:
        return ta
    lane = jax.lax.broadcasted_iota(i32, ta.shape, 1)
    return jnp.where(lane >= off, ta, a[t0 + 1])


def _swiglu(g, u):
    hg = 0.5 * g
    p = hg * u
    return p + p * jnp.tanh(hg)


def _attn_fns(first, blk, q_ref, k_ref, vt_ref, ot_ref, s_ref, p_ref, tokens):
    lane16 = jax.lax.broadcasted_iota(i32, (16, 128), 1)
    row16 = jax.lax.broadcasted_iota(i32, (16, 128), 0)
    lane32 = jax.lax.broadcasted_iota(i32, (32, 128), 1)
    row32 = jax.lax.broadcasted_iota(i32, (32, 128), 0)
    tri = row32 <= (lane32 % 32)
    b0 = (lane16 & 32) == 0
    b1 = (lane16 & 64) == 0
    b0_24 = (jax.lax.broadcasted_iota(i32, (24, 128), 1) & 32) == 0
    zero16 = jnp.zeros((16, 128), i32)
    pi_ref = p_ref.bitcast(i32)
    zs = jax.lax.shift_right_logical(pl.program_id(0), 6)
    dz = pl.multiple_of(zs * 8, 8)

    def miss_of(qb):
        return max(8 - 4 * qb, 0) if first else 0

    def qk(slot, qb, g):
        miss = miss_of(qb)
        masks = []
        for h in range(4):
            lo = (80 * g + 20 * h) % 128
            if lo + 20 <= 128:
                msk = (lane16 >= lo) & (lane16 < lo + 20)
            else:
                msk = (lane16 >= lo) | (lane16 < lo + 20 - 128)
            masks.append(jnp.where(msk, -1, 0))
        mxs = []
        for j in range(4):
            q = q_ref[g, qb * 64 + 16 * j: qb * 64 + 16 * j + 16, :]
            wq = pltpu.bitcast(jnp.concatenate([q & masks[m ^ j] for m in range(4)], axis=0), bf16)
            c0 = max(j, miss)
            nrows = (j + 9 - c0) * 32
            if first:
                r0 = qb * 64 + 16 * c0
                kk = k_ref[g, r0: r0 + nrows // 2, :]
            else:
                kk = k_ref[g, pl.ds(pl.multiple_of(blk * (T // 2) + qb * 64 + 16 * c0, 16), nrows // 2), :]
            s = jax.lax.dot_general(pltpu.bitcast(kk, bf16), wq, NT, preferred_element_type=f32)
            if j == 3:
                tokens[:] = [s[(r * nrows // 256) // 8 * 8:(r * nrows // 256) // 8 * 8 + 8] for r in TOK]
            bot = s[nrows - 32:, :]
            if c0 == j:
                sm = jnp.where(tri, bot, s[:32, :])
                mid = s[32:nrows - 32, :]
            else:
                sm = jnp.where(tri, bot, float('-inf'))
                mid = s[:nrows - 32, :] if nrows > 32 else None
            allm = sm if mid is None else jnp.concatenate([mid, sm], axis=0)
            n = allm.shape[0]
            s_ref[slot][256 * j + 256 - n:256 * j + 256, :] = allm
            parts = [allm[8 * t:8 * t + 8] for t in range(n // 8)]
            accs = parts[:4]
            for t in range(4, len(parts)):
                accs[t % 4] = jnp.maximum(accs[t % 4], parts[t])
            m8 = jnp.maximum(jnp.maximum(accs[0], accs[1]), jnp.maximum(accs[2], accs[3]))
            mx = jnp.max(m8, axis=0, keepdims=True)
            mxs.append(jnp.broadcast_to(mx, (8, 128)))
        return dict(slot=slot, qb=qb, g=g, mxs=mxs, R=[None] * 4, pm={}, Z={})

    def exp_tile(st, t):
        slot, qb, mxs = st['slot'], st['qb'], st['mxs']
        if 4 * t < miss_of(qb):
            return
        Z = [[] for _ in range(4)]
        for c in range(4 * t, 4 * t + 4):
            zero = None if first else pltpu.bitcast(pltpu.bitcast(tokens[c % 4], i32) & zs, f32)

            def ex(j, r0):
                m = mxs[j] if zero is None else mxs[j] + zero
                sv = s_ref[slot][pl.ds(dz + 256 * j + r0, 32), :]
                return jnp.exp2(sv - jnp.concatenate([m] * 4, axis=0))

            def pk(j):
                if c < j or c > j + 8:
                    return None
                if c == j or c == j + 8:
                    if j not in st['pm']:
                        st['pm'][j] = ex(j, 224)
                    pm = st['pm'][j]
                    v = jnp.where(tri, 0.0, pm) if c == j else jnp.where(tri, pm, 0.0)
                else:
                    v = ex(j, 32 * (c - j - 1))
                p_ref[32 * j:32 * j + 32, :] = v.astype(bf16)
                return pi_ref[16 * j:16 * j + 16, :]

            def sel(mask, a, b):
                if a is None and b is None:
                    return None
                return jnp.where(mask, zero16 if a is None else a, zero16 if b is None else b)
            X = [pk(j) for j in range(4)]
            Y = [[sel(b0, X[2 * j1], X[2 * j1 + 1]), sel(b0, X[2 * j1 + 1], X[2 * j1])] for j1 in range(2)]
            for h0 in range(2):
                Z[h0].append(sel(b1, Y[0][h0], Y[1][h0]))
                Z[2 + h0].append(sel(b1, Y[1][h0], Y[0][h0]))
        st['Z'][t] = Z

    def mm_tiles(st, tl):
        qb, g = st['qb'], st['g']
        last = 2 in tl
        tl = [u for u in tl if u in st['Z']]
        if tl:
            for h in range(4):
                hh = 4 * g + h
                w0 = (20 * hh) // 16 * 16
                o = 20 * hh - w0
                vs = []
                for u in tl:
                    v = vt_ref[blk * 2 + qb + u, w0 // 2:w0 // 2 + 16, :]
                    ones_rows = (row16 >= 12) if o < 8 else (row16 < 4)
                    vs.append(jnp.where(ones_rows, ONES_PK, v))
                v = pltpu.bitcast(jnp.concatenate(vs, axis=1) if len(vs) > 1 else vs[0], bf16)
                ph = pltpu.bitcast(jnp.concatenate(sum([st['Z'][u][h] for u in tl], []), axis=0), bf16)
                r = jnp.dot(v, ph, preferred_element_type=f32)
                st['R'][h] = r if st['R'][h] is None else st['R'][h] + r
        if last:
            outs = []
            for h in range(4):
                o = (20 * h) % 16
                r = st['R'][h]
                if o < 8:
                    l8, dat = r[24:32, :], r[0:24, :]
                else:
                    l8, dat = r[0:8, :], r[8:32, :]
                inv = pl.reciprocal(l8, approx=True)
                inv = inv * (2.0 - l8 * inv)
                dat = dat * jnp.concatenate([inv, inv, inv], axis=0)
                if h == 1:
                    dat = jnp.where(b0_24, pltpu.roll(dat, 96, 1), pltpu.roll(dat, 32, 1))
                elif h == 2:
                    dat = pltpu.roll(dat, 64, 1)
                elif h == 3:
                    dat = jnp.where(b0_24, pltpu.roll(dat, 32, 1), pltpu.roll(dat, 96, 1))
                outs.append(dat)
            sub = jax.lax.broadcasted_iota(i32, (8, 128), 0)
            og = jnp.concatenate([
                outs[0][0:16], jnp.where(sub < 4, outs[0][16:24], outs[1][0:8]), outs[1][8:24],
                outs[2][0:16], jnp.where(sub < 4, outs[2][16:24], outs[3][0:8]), outs[3][8:24]], axis=0)
            ot_ref[qb, 80 * g:80 * g + 80, :] = og
    return qk, exp_tile, mm_tiles


def _kernel(x_hbm, wqkv_hbm, wo_hbm, w1t_hbm, w3t_hbm, w2_hbm, o_hbm,
            x_ref, wqkv_ref, wvt_ref, wo_ref, w13_ref, w2_ref, q0, q1, k_ref, vt_ref, ot0, ot1,
            s0, s1, s2, h_ref, hn_ref, xn_ref, p0, p1, o_ref, sems, osem):
    s_ref = [s0, s1, s2]
    s_id = pl.program_id(0)

    def xrest():
        return pltpu.make_async_copy(x_hbm.at[4:NB], x_ref.at[4:NB], sems.at[7])

    class FFN:
        def __init__(self, tokens):
            self.tokens = tokens
            self.blk = s_id - 1
            self.jobs = [('up', n) for n in range(27)] + [('down', n) for n in range(5)]
            self.k = 0
            self.acc = None
            self.gate = None
            self.acts = []
            self.left = 27 * 5 + 5 * 14

        def emit(self, npass):
            npass = min(npass, self.left)
            self.left -= npass
            while npass > 0:
                kind, n = self.jobs[0]
                kt = 5 if kind == 'up' else 14
                m = min(npass, kt - self.k)
                k0, k1 = self.k, self.k + m
                if kind == 'up':
                    lhs = pltpu.bitcast(hn_ref[self.blk & 1, :, 128 * k0:128 * k1], bf16)
                    if n < 26:
                        c = n // 2
                        w = w13_ref[n % 2, 128 * c:128 * c + 128, 128 * k0:128 * k1]
                    else:
                        w = jnp.concatenate([w13_ref[0, 1664:1728, 128 * k0:128 * k1],
                                             w13_ref[1, 1664:1728, 128 * k0:128 * k1]], axis=0)
                    r = jax.lax.dot_general(lhs, w, NT, preferred_element_type=f32)
                else:
                    r = None
                    for c in range(k0, k1):
                        kw = 128 if c < 13 else 64
                        rr = jnp.dot(self.acts[c], w2_ref[128 * c:128 * c + kw, 128 * n:128 * n + 128],
                                     preferred_element_type=f32)
                        r = rr if r is None else r + rr
                self.acc = r if self.acc is None else self.acc + r
                self.tokens[:] = [self.acc[r0:r0 + 8] for r0 in TOK]
                self.k = k1
                npass -= m
                if self.k == kt:
                    if kind == 'down':
                        o_ref[self.blk, n] = (h_ref[self.blk & 3, :, 128 * n:128 * n + 128] + self.acc).astype(bf16)
                        pltpu.make_async_copy(o_ref.at[self.blk, n],
                                              o_hbm.at[self.blk, :, 128 * n:128 * n + 128], osem.at[0]).start()
                    elif n == 26:
                        a = _swiglu(self.acc, pltpu.roll(self.acc, 64, 1))
                        self.acts.append(a[:, :64].astype(bf16))
                    elif n % 2 == 0:
                        self.gate = self.acc
                    else:
                        self.acts.append(_swiglu(self.gate, self.acc).astype(bf16))
                    self.acc = None
                    self.k = 0
                    self.jobs.pop(0)

    def qk_tiles(xn, a, b):
        r = jnp.dot(xn, wqkv_ref[:, 128 * a:128 * b], preferred_element_type=f32)
        out = []
        for t in range(a, b):
            v = r[:, 128 * (t - a):128 * (t - a + 1)]
            if t < 5:
                v = v * (DH ** -0.5 * LOG2E)
            out.append(pltpu.bitcast(v.astype(bf16), i32))
        return out

    def store_qk(first, tiles, blk):
        hT = T // 2
        for g in range(NG):
            if first:
                q0[g, blk * hT:blk * hT + hT, :] = _group_tile(tiles[:5], g)
            else:
                q1[g] = _group_tile(tiles[:5], g)
        for g in range(NG):
            kg = _group_tile(tiles[5:], g)
            if first:
                k_ref[g, W // 2 + blk * hT:W // 2 + blk * hT + hT, :] = kg
            else:
                k_ref[g, pl.ds(pl.multiple_of(W // 2 + blk * hT, hT), hT), :] = kg

    def store_vt(xn, blk):
        for u in range(2):
            vt = jax.lax.dot_general(wvt_ref[320 * u:320 * u + 320, :], xn, NT, preferred_element_type=f32)
            vt = pltpu.bitcast(vt.astype(bf16), i32)
            for t in range(2):
                vt_ref[2 + blk * 2 + t, 160 * u:160 * u + 160, :] = vt[:, t * 128:(t + 1) * 128]

    def run_attn(first, nq, blk, dep, pats, filler, tokens):
        qk, exp_tile, mm_tiles = _attn_fns(first, blk, q0 if first else q1, k_ref, vt_ref,
                                           ot0 if first else ot1, s_ref, p0 if first else p1, tokens)
        items = [(qb, g) for qb in range(nq) for g in range(NG)]
        n = len(items)
        ss = {}
        for t in range(dep):
            ss[t] = qk(t % (dep + 1), *items[t])
        for t in range(n + 1):
            pat = pats[min(t, n - 1)]
            for p, ch in enumerate(pat):
                if ch == 'w':
                    if t > 0:
                        mm_tiles(ss[t - 1], [0, 1, 2])
                elif t == n or ch.isdigit():
                    pass
                elif ch == 'F':
                    filler.emit(int(pat[p + 1]))
                elif ch == 'J':
                    filler(t)
                elif ch == 'q':
                    if t + dep < n:
                        ss[t + dep] = qk((t + dep) % (dep + 1), *items[t + dep])
                elif ch in 'abc':
                    exp_tile(ss[t], 'abc'.index(ch))
                else:
                    mm_tiles(ss[t], ['ABC'.index(ch)])
            if t == n - 1 and 'w' in pat:
                filler.emit(4)

    def wo_proj(x, ot_ref, qbs):
        o = [ot_ref[qb].T for qb in qbs]
        o = jnp.concatenate(o, axis=0) if len(o) > 1 else o[0]
        return x + jnp.dot(o.astype(bf16), wo_ref[...], preferred_element_type=f32)

    @pl.when(s_id == 0)
    def _():
        def hcopy(src, dst, k):
            return pltpu.make_async_copy(src, dst, sems.at[k])

        def wcol(a, b, k):
            return hcopy(wqkv_hbm.at[:, a:b], wqkv_ref.at[:, a:b], k)
        cx0, cx1 = hcopy(x_hbm.at[0], x_ref.at[0], 0), hcopy(x_hbm.at[1], x_ref.at[1], 1)
        ca = wcol(0, 256, 2)
        cb = wcol(256, 768, 3)
        cc = [wcol(2 * D, 3 * D, 4), wcol(768, 1024, 4)]
        cd = [wcol(1024, 1280, 5), hcopy(wo_hbm, wo_ref, 5), hcopy(x_hbm.at[2], x_ref.at[2], 5)]
        ce = [hcopy(x_hbm.at[3], x_ref.at[3], 6), hcopy(w1t_hbm, w13_ref.at[0], 6),
              hcopy(w3t_hbm, w13_ref.at[1], 6), hcopy(w2_hbm, w2_ref, 6)]
        for c in [cx0, cx1, ca, cb] + cc + cd + ce + [xrest()]:
            c.start()
        cx0.wait()
        xn0 = _ln(x_ref[0].astype(f32))
        cx1.wait()
        xn1 = _ln(x_ref[1].astype(f32))
        xn = jnp.concatenate([xn0, xn1], axis=0).astype(bf16)
        xh = [xn[:T], xn[T:]]
        tiles = [[], []]

        def split_tiles(a, b, blks=(0, 1)):
            for u in blks:
                tiles[u] += qk_tiles(xh[u], a, b)
        ca.wait()
        split_tiles(0, 2)
        cb.wait()
        for tl in qk_tiles(xn, 2, 6):
            tiles[0].append(tl[:T // 2])
            tiles[1].append(tl[T // 2:])
        for c in cc:
            c.wait()
        wvt_ref[...] = wqkv_ref[:, 2 * D:].astype(f32).T.astype(bf16)
        split_tiles(6, 8)
        store_vt(xh[0], 0)

        def vjob(u, t):
            def run():
                vt = jax.lax.dot_general(wvt_ref[320 * u:320 * u + 320, :], xh[1][128 * t:128 * t + 128], NT,
                                         preferred_element_type=f32)
                vt_ref[4 + t, 160 * u:160 * u + 160, :] = pltpu.bitcast(vt.astype(bf16), i32)
            return run

        def kjob(t):
            def run():
                split_tiles(t, t + 1, (1,))
                if t == 9:
                    store_qk(True, tiles[1], 1)
            return run
        jobs = [kjob(8), kjob(9)] + [vjob(u, t) for t in range(2) for u in range(2)]
        for c in cd:
            c.wait()
        split_tiles(8, 10, (0,))
        store_qk(True, tiles[0], 0)
        run_attn(True, 4, 0, 2, [PAT_FIRST_FILL if t in FILL_AT else PAT_FIRST for t in range(32)],
                 lambda t: jobs.pop(0)(), [])
        assert not jobs
        hs = []
        for qb in range(4):
            blk, half = qb // 2, qb % 2
            h = wo_proj(x_ref[blk, 128 * half:128 * half + 128, :].astype(f32), ot0, [qb])
            h_ref[blk, 128 * half:128 * half + 128, :] = h
            hs.append(h)
        xn_ref[...] = pltpu.bitcast(_ln(x_ref[2].astype(f32)).astype(bf16), i32)
        for qb in range(4):
            blk, half = qb // 2, qb % 2
            hn_ref[blk, 64 * half:64 * half + 64, :] = pltpu.bitcast(_ln(hs[qb]).astype(bf16), i32)
        for c in ce:
            c.wait()

    @pl.when(s_id == 2)
    def _():
        xrest().wait()

    @pl.when((s_id > 0) & (s_id < NB - 1))
    def _():
        blk = s_id + 1
        tokens = []
        ffn = FFN(tokens)
        zs = jax.lax.shift_right_logical(s_id, 6)

        def paced(plan):
            zeros = []
            for npass in plan:
                ffn.emit(npass)
                zeros += [pltpu.bitcast(pltpu.bitcast(tk, i32) & zs, f32) for tk in tokens]
            return zeros
        xn = pltpu.bitcast(xn_ref[...], bf16)
        store_qk(False, qk_tiles(xn, 0, 10), blk)
        ffn.emit(6)
        store_vt(xn, blk)
        run_attn(False, 2, blk, 1, [PAT_MID] * 16, ffn, tokens)
        ffn.emit(8)
        h = wo_proj(x_ref[blk].astype(f32), ot1, [0, 1])
        h_ref[blk & 3] = h
        assert ffn.left <= 70
        z2 = paced((8, 8))
        hn_ref[blk & 1] = pltpu.bitcast(_ln(h, z2).astype(bf16), i32)
        z1 = paced((8, 8))
        xn_ref[...] = pltpu.bitcast(_ln(x_ref[jnp.minimum(blk + 1, NB - 1)].astype(f32), z1).astype(bf16), i32)
        ffn.emit(1000)

    @pl.when(s_id >= NB - 1)
    def _():
        FFN([]).emit(1000)

    @pl.when(s_id == NB)
    def _():
        pltpu.make_async_copy(o_ref, o_ref, osem.at[0]).wait()


@jax.jit
def pallas_sequential_preLN__sliding_block__glu_gated_swiglu__prompt_kernel(
    A_x: jax.Array,
    A_wqkv: jax.Array,
    A_wo: jax.Array,
    B_x: jax.Array,
    B_w1: jax.Array,
    B_w3: jax.Array,
    B_w2: jax.Array,
):
    anyspec = pl.BlockSpec(memory_space=pl.ANY)
    out = pl.pallas_call(
        _kernel,
        out_shape=jax.ShapeDtypeStruct((NB, T, D), bf16),
        grid=(NB + 1,),
        in_specs=[anyspec] * 6,
        out_specs=anyspec,
        scratch_shapes=[
            pltpu.VMEM((NB, T, D), bf16),
            pltpu.VMEM((D, 3 * D), bf16),
            pltpu.VMEM((D, D), bf16),
            pltpu.VMEM((D, D), bf16),
            pltpu.VMEM((2, F, D), bf16),
            pltpu.VMEM((F, D), bf16),
            pltpu.VMEM((NG, T, 128), i32),
            pltpu.VMEM((NG, T // 2, 128), i32),
            pltpu.VMEM((NG, (W + S) // 2, 128), i32),
            pltpu.VMEM((2 + S // 128, D // 2, 128), i32),
            pltpu.VMEM((4, D, 128), f32),
            pltpu.VMEM((2, D, 128), f32),
            pltpu.VMEM((1024, 128), f32),
            pltpu.VMEM((1024, 128), f32),
            pltpu.VMEM((1024, 128), f32),
            pltpu.VMEM((4, T, D), f32),
            pltpu.VMEM((2, T // 2, D), i32),
            pltpu.VMEM((T // 2, D), i32),
            pltpu.VMEM((128, 128), bf16),
            pltpu.VMEM((128, 128), bf16),
            pltpu.VMEM((NB, 5, T, 128), bf16),
            pltpu.SemaphoreType.DMA((8,)),
            pltpu.SemaphoreType.DMA((1,)),
        ],
        compiler_params=pltpu.CompilerParams(dimension_semantics=("arbitrary",),
                                             vmem_limit_bytes=100 * 1024 * 1024,
                                             disable_bounds_checks=True),
    )(A_x.reshape(NB, T, D), A_wqkv, A_wo, B_w1.T, B_w3.T, B_w2)
    return out.reshape(1, S, D)
```

```python
import jax
import jax.numpy as jnp
import jax.experimental.pallas as pl
import jax.experimental.pallas.tpu as pltpu

S, D, F = 2048, 640, 1728
H, DH, W = 32, 20, 256
NG = 8
T = 256
NB = S // T
LOG2E = 1.4426950408889634
f32 = jnp.float32
bf16 = jnp.bfloat16
i32 = jnp.int32
NT = (((1,), (1,)), ((), ()))
ONES_PK = 0x3F803F80

PAT_FIRST, PAT_FIRST_FILL, FILL_AT = "qaAbBcC", "qaJAbBcC", (0, 1, 2, 5, 8, 10)
PAT_MID = "qaF4wbF4c"
TOK = (40, 104, 168, 232)


def _ln(x, zeros=None):
    m = jnp.mean(x, axis=-1, keepdims=True)
    if zeros:
        rep = x.shape[0] // (8 * len(zeros))
        m = m + jnp.concatenate([z[:, :1] for z in zeros for _ in range(rep)], axis=0)
    mb = m.astype(bf16).astype(f32)
    xc = x - mb
    dm = m - mb
    ve = jnp.maximum(jnp.mean(xc * xc, axis=-1, keepdims=True) + (1e-5 - dm * dm), 1e-5)
    return xc * jax.lax.rsqrt(ve)


def _group_tile(a, g):
    lo = 80 * g
    t0, off = lo // 128, lo % 128
    ta = a[t0]
    if off + 80 <= 128:
        return ta
    lane = jax.lax.broadcasted_iota(i32, ta.shape, 1)
    return jnp.where(lane >= off, ta, a[t0 + 1])


def _swiglu(g, u):
    hg = 0.5 * g
    p = hg * u
    return p + p * jnp.tanh(hg)


def _pack_pairs(b, clear_low):
    outs = []
    for u in range(b.shape[0] // 16):
        hi = b[16 * u + 8:16 * u + 16]
        outs.append(jax.lax.shift_right_logical(b[16 * u:16 * u + 8], 16) | ((hi & (-65536)) if clear_low else hi))
    return jnp.concatenate(outs, axis=0)


def _attn_fns(first, blk, q_ref, k_ref, vt_ref, ot_ref, s_ref, tokens):
    lane16 = jax.lax.broadcasted_iota(i32, (16, 128), 1)
    row16 = jax.lax.broadcasted_iota(i32, (16, 128), 0)
    lane32 = jax.lax.broadcasted_iota(i32, (32, 128), 1)
    row32 = jax.lax.broadcasted_iota(i32, (32, 128), 0)
    tri = row32 <= (lane32 % 32)
    b0 = (lane16 & 32) == 0
    b1 = (lane16 & 64) == 0
    b0_24 = (jax.lax.broadcasted_iota(i32, (24, 128), 1) & 32) == 0
    zero16 = jnp.zeros((16, 128), i32)
    zs = jax.lax.shift_right_logical(pl.program_id(0), 6)
    dz = pl.multiple_of(zs * 8, 8)

    prow = (row16 & 7) + (row16 >> 3) * 16
    tri_pk = (jnp.where(prow <= (lane16 % 32), 65535, 0) | jnp.where(prow + 8 <= (lane16 % 32), -65536, 0))

    def miss_of(qb):
        return max(8 - 4 * qb, 0) if first else 0

    def qk(slot, qb, g):
        miss = miss_of(qb)
        masks = []
        for h in range(4):
            lo = (80 * g + 20 * h) % 128
            if lo + 20 <= 128:
                msk = (lane16 >= lo) & (lane16 < lo + 20)
            else:
                msk = (lane16 >= lo) | (lane16 < lo + 20 - 128)
            masks.append(jnp.where(msk, -1, 0))
        mxs = []
        for j in range(4):
            q = q_ref[g, qb * 64 + 16 * j: qb * 64 + 16 * j + 16, :]
            wq = pltpu.bitcast(jnp.concatenate([q & masks[m ^ j] for m in range(4)], axis=0), bf16)
            c0 = max(j, miss)
            nrows = (j + 9 - c0) * 32
            if first:
                r0 = qb * 64 + 16 * c0
                kk = k_ref[g, r0: r0 + nrows // 2, :]
            else:
                kk = k_ref[g, pl.ds(pl.multiple_of(blk * (T // 2) + qb * 64 + 16 * c0, 16), nrows // 2), :]
            s = jax.lax.dot_general(pltpu.bitcast(kk, bf16), wq, NT, preferred_element_type=f32)
            if j == 3:
                tokens[:] = [s[(r * nrows // 256) // 8 * 8:(r * nrows // 256) // 8 * 8 + 8] for r in TOK]
            bot = s[nrows - 32:, :]
            if c0 == j:
                sm = jnp.where(tri, bot, s[:32, :])
                mid = s[32:nrows - 32, :]
            else:
                sm = jnp.where(tri, bot, float('-inf'))
                mid = s[:nrows - 32, :] if nrows > 32 else None
            allm = sm if mid is None else jnp.concatenate([mid, sm], axis=0)
            n = allm.shape[0]
            s_ref[slot][256 * j + 256 - n:256 * j + 256, :] = allm
            parts = [allm[8 * t:8 * t + 8] for t in range(n // 8)]
            accs = parts[:4]
            for t in range(4, len(parts)):
                accs[t % 4] = jnp.maximum(accs[t % 4], parts[t])
            m8 = jnp.maximum(jnp.maximum(accs[0], accs[1]), jnp.maximum(accs[2], accs[3]))
            mx = jnp.max(m8, axis=0, keepdims=True)
            mxs.append(jnp.broadcast_to(mx, (8, 128)))
        return dict(slot=slot, qb=qb, g=g, mxs=mxs, R=[None] * 4, pm={}, Z={})

    def exp_tile(st, t):
        slot, qb, mxs = st['slot'], st['qb'], st['mxs']
        if 4 * t < miss_of(qb):
            return
        Z = [[] for _ in range(4)]
        for c in range(4 * t, 4 * t + 4):
            zero = None if first else pltpu.bitcast(pltpu.bitcast(tokens[c % 4], i32) & zs, f32)

            def ex(j, r0):
                m = mxs[j] if zero is None else mxs[j] + zero
                sv = s_ref[slot][pl.ds(dz + 256 * j + r0, 32), :]
                p = jnp.exp2(sv - jnp.concatenate([m] * 4, axis=0))
                return _pack_pairs(pltpu.bitcast(p, i32), True)

            def pk(j):
                if c < j or c > j + 8:
                    return None
                if c == j or c == j + 8:
                    if j not in st['pm']:
                        st['pm'][j] = ex(j, 224)
                    return st['pm'][j] & (~tri_pk if c == j else tri_pk)
                return ex(j, 32 * (c - j - 1))

            def sel(mask, a, b):
                if a is None and b is None:
                    return None
                return jnp.where(mask, zero16 if a is None else a, zero16 if b is None else b)
            X = [pk(j) for j in range(4)]
            Y = [[sel(b0, X[2 * j1], X[2 * j1 + 1]), sel(b0, X[2 * j1 + 1], X[2 * j1])] for j1 in range(2)]
            for h0 in range(2):
                Z[h0].append(sel(b1, Y[0][h0], Y[1][h0]))
                Z[2 + h0].append(sel(b1, Y[1][h0], Y[0][h0]))
        st['Z'][t] = Z

    def mm_tiles(st, tl):
        qb, g = st['qb'], st['g']
        last = 2 in tl
        tl = [u for u in tl if u in st['Z']]
        if tl:
            for h in range(4):
                hh = 4 * g + h
                w0 = (20 * hh) // 16 * 16
                o = 20 * hh - w0
                vs = []
                for u in tl:
                    v = vt_ref[blk * 2 + qb + u, w0 // 2:w0 // 2 + 16, :]
                    ones_rows = (row16 >= 12) if o < 8 else (row16 < 4)
                    vs.append(jnp.where(ones_rows, ONES_PK, v))
                v = pltpu.bitcast(jnp.concatenate(vs, axis=1) if len(vs) > 1 else vs[0], bf16)
                ph = pltpu.bitcast(jnp.concatenate(sum([st['Z'][u][h] for u in tl], []), axis=0), bf16)
                r = jnp.dot(v, ph, preferred_element_type=f32)
                st['R'][h] = r if st['R'][h] is None else st['R'][h] + r
        if last:
            outs = []
            for h in range(4):
                o = (20 * h) % 16
                r = st['R'][h]
                if o < 8:
                    l8, dat = r[24:32, :], r[0:24, :]
                else:
                    l8, dat = r[0:8, :], r[8:32, :]
                inv = pl.reciprocal(l8, approx=True)
                inv = inv * (2.0 - l8 * inv)
                dat = dat * jnp.concatenate([inv, inv, inv], axis=0)
                if h == 1:
                    dat = jnp.where(b0_24, pltpu.roll(dat, 96, 1), pltpu.roll(dat, 32, 1))
                elif h == 2:
                    dat = pltpu.roll(dat, 64, 1)
                elif h == 3:
                    dat = jnp.where(b0_24, pltpu.roll(dat, 32, 1), pltpu.roll(dat, 96, 1))
                outs.append(dat)
            sub = jax.lax.broadcasted_iota(i32, (8, 128), 0)
            og = jnp.concatenate([
                outs[0][0:16], jnp.where(sub < 4, outs[0][16:24], outs[1][0:8]), outs[1][8:24],
                outs[2][0:16], jnp.where(sub < 4, outs[2][16:24], outs[3][0:8]), outs[3][8:24]], axis=0)
            ot_ref[qb, 80 * g:80 * g + 80, :] = og
    return qk, exp_tile, mm_tiles


def _kernel(x_hbm, wqkv_hbm, wo_hbm, w1t_hbm, w3t_hbm, w2_hbm, o_hbm,
            x_ref, wqkv_ref, wvt_ref, wo_ref, w13_ref, w2_ref, q0, q1, k_ref, vt_ref, ot0, ot1,
            s0, s1, s2, h_ref, hn_ref, xn_ref, o_ref, sems, osem):
    s_ref = [s0, s1, s2]
    s_id = pl.program_id(0)

    def xrest():
        return pltpu.make_async_copy(x_hbm.at[4:NB], x_ref.at[4:NB], sems.at[7])

    class FFN:
        def __init__(self, tokens):
            self.tokens = tokens
            self.blk = s_id - 1
            self.jobs = [('up', n) for n in range(27)] + [('down', n) for n in range(5)]
            self.k = 0
            self.acc = None
            self.gate = None
            self.acts = []
            self.left = 27 * 5 + 5 * 14

        def emit(self, npass):
            npass = min(npass, self.left)
            self.left -= npass
            while npass > 0:
                kind, n = self.jobs[0]
                kt = 5 if kind == 'up' else 14
                m = min(npass, kt - self.k)
                k0, k1 = self.k, self.k + m
                if kind == 'up':
                    lhs = pltpu.bitcast(hn_ref[self.blk & 1, :, 128 * k0:128 * k1], bf16)
                    if n < 26:
                        c = n // 2
                        w = w13_ref[n % 2, 128 * c:128 * c + 128, 128 * k0:128 * k1]
                    else:
                        w = jnp.concatenate([w13_ref[0, 1664:1728, 128 * k0:128 * k1],
                                             w13_ref[1, 1664:1728, 128 * k0:128 * k1]], axis=0)
                    r = jax.lax.dot_general(lhs, w, NT, preferred_element_type=f32)
                else:
                    r = None
                    for c in range(k0, k1):
                        kw = 128 if c < 13 else 64
                        rr = jnp.dot(self.acts[c], w2_ref[128 * c:128 * c + kw, 128 * n:128 * n + 128],
                                     preferred_element_type=f32)
                        r = rr if r is None else r + rr
                self.acc = r if self.acc is None else self.acc + r
                self.tokens[:] = [self.acc[r0:r0 + 8] for r0 in TOK]
                self.k = k1
                npass -= m
                if self.k == kt:
                    if kind == 'down':
                        o_ref[self.blk, n] = (h_ref[self.blk & 3, :, 128 * n:128 * n + 128] + self.acc).astype(bf16)
                        pltpu.make_async_copy(o_ref.at[self.blk, n],
                                              o_hbm.at[self.blk, :, 128 * n:128 * n + 128], osem.at[0]).start()
                    elif n == 26:
                        a = _swiglu(self.acc, pltpu.roll(self.acc, 64, 1))
                        self.acts.append(a[:, :64].astype(bf16))
                    elif n % 2 == 0:
                        self.gate = self.acc
                    else:
                        self.acts.append(_swiglu(self.gate, self.acc).astype(bf16))
                    self.acc = None
                    self.k = 0
                    self.jobs.pop(0)

    def qk_tiles(xn, a, b):
        r = jnp.dot(xn, wqkv_ref[:, 128 * a:128 * b], preferred_element_type=f32)
        out = []
        for t in range(a, b):
            v = r[:, 128 * (t - a):128 * (t - a + 1)]
            if t < 5:
                v = v * (DH ** -0.5 * LOG2E)
            out.append(pltpu.bitcast(v.astype(bf16), i32))
        return out

    def store_qk(first, tiles, blk):
        hT = T // 2
        for g in range(NG):
            if first:
                q0[g, blk * hT:blk * hT + hT, :] = _group_tile(tiles[:5], g)
            else:
                q1[g] = _group_tile(tiles[:5], g)
        for g in range(NG):
            kg = _group_tile(tiles[5:], g)
            if first:
                k_ref[g, W // 2 + blk * hT:W // 2 + blk * hT + hT, :] = kg
            else:
                k_ref[g, pl.ds(pl.multiple_of(W // 2 + blk * hT, hT), hT), :] = kg

    def perm(xn):
        return pltpu.bitcast(_pack_pairs(pltpu.bitcast(xn.astype(f32), i32), False), bf16)

    def store_vt(xn, blk):
        xn = perm(xn)
        for u in range(2):
            vt = jax.lax.dot_general(wvt_ref[320 * u:320 * u + 320, :], xn, NT, preferred_element_type=f32)
            vt = pltpu.bitcast(vt.astype(bf16), i32)
            for t in range(2):
                vt_ref[2 + blk * 2 + t, 160 * u:160 * u + 160, :] = vt[:, t * 128:(t + 1) * 128]

    def run_attn(first, nq, blk, dep, pats, filler, tokens):
        qk, exp_tile, mm_tiles = _attn_fns(first, blk, q0 if first else q1, k_ref, vt_ref,
                                           ot0 if first else ot1, s_ref, tokens)
        items = [(qb, g) for qb in range(nq) for g in range(NG)]
        n = len(items)
        ss = {}
        for t in range(dep):
            ss[t] = qk(t % (dep + 1), *items[t])
        for t in range(n + 1):
            pat = pats[min(t, n - 1)]
            for p, ch in enumerate(pat):
                if ch == 'w':
                    if t > 0:
                        mm_tiles(ss[t - 1], [0, 1, 2])
                elif t == n or ch.isdigit():
                    pass
                elif ch == 'F':
                    filler.emit(int(pat[p + 1]))
                elif ch == 'J':
                    filler(t)
                elif ch == 'q':
                    if t + dep < n:
                        ss[t + dep] = qk((t + dep) % (dep + 1), *items[t + dep])
                elif ch in 'abc':
                    exp_tile(ss[t], 'abc'.index(ch))
                else:
                    mm_tiles(ss[t], ['ABC'.index(ch)])
            if t == n - 1 and 'w' in pat:
                filler.emit(4)

    def wo_proj(x, ot_ref, qbs):
        o = [ot_ref[qb].T for qb in qbs]
        o = jnp.concatenate(o, axis=0) if len(o) > 1 else o[0]
        return x + jnp.dot(o.astype(bf16), wo_ref[...], preferred_element_type=f32)

    @pl.when(s_id == 0)
    def _():
        def hcopy(src, dst, k):
            return pltpu.make_async_copy(src, dst, sems.at[k])

        def wcol(a, b, k):
            return hcopy(wqkv_hbm.at[:, a:b], wqkv_ref.at[:, a:b], k)
        cx0, cx1 = hcopy(x_hbm.at[0], x_ref.at[0], 0), hcopy(x_hbm.at[1], x_ref.at[1], 1)
        ca = wcol(0, 256, 2)
        cb = wcol(256, 768, 3)
        cc = [wcol(2 * D, 3 * D, 4), wcol(768, 1024, 4)]
        cd = [wcol(1024, 1280, 5), hcopy(wo_hbm, wo_ref, 5), hcopy(x_hbm.at[2], x_ref.at[2], 5)]
        ce = [hcopy(x_hbm.at[3], x_ref.at[3], 6), hcopy(w1t_hbm, w13_ref.at[0], 6),
              hcopy(w3t_hbm, w13_ref.at[1], 6), hcopy(w2_hbm, w2_ref, 6)]
        for c in [cx0, cx1, ca, cb] + cc + cd + ce + [xrest()]:
            c.start()
        cx0.wait()
        xn0 = _ln(x_ref[0].astype(f32))
        cx1.wait()
        xn1 = _ln(x_ref[1].astype(f32))
        xn = jnp.concatenate([xn0, xn1], axis=0).astype(bf16)
        xh = [xn[:T], xn[T:]]
        tiles = [[], []]

        def split_tiles(a, b, blks=(0, 1)):
            for u in blks:
                tiles[u] += qk_tiles(xh[u], a, b)
        ca.wait()
        split_tiles(0, 2)
        cb.wait()
        for tl in qk_tiles(xn, 2, 6):
            tiles[0].append(tl[:T // 2])
            tiles[1].append(tl[T // 2:])
        for c in cc:
            c.wait()
        wvt_ref[...] = wqkv_ref[:, 2 * D:].astype(f32).T.astype(bf16)
        split_tiles(6, 8)
        store_vt(xh[0], 0)

        def vjob(u, t):
            def run():
                vt = jax.lax.dot_general(wvt_ref[320 * u:320 * u + 320, :], perm(xh[1][128 * t:128 * t + 128]), NT,
                                         preferred_element_type=f32)
                vt_ref[4 + t, 160 * u:160 * u + 160, :] = pltpu.bitcast(vt.astype(bf16), i32)
            return run

        def kjob(t):
            def run():
                split_tiles(t, t + 1, (1,))
                if t == 9:
                    store_qk(True, tiles[1], 1)
            return run
        jobs = [kjob(8), kjob(9)] + [vjob(u, t) for t in range(2) for u in range(2)]
        for c in cd:
            c.wait()
        split_tiles(8, 10, (0,))
        store_qk(True, tiles[0], 0)
        run_attn(True, 4, 0, 2, [PAT_FIRST_FILL if t in FILL_AT else PAT_FIRST for t in range(32)],
                 lambda t: jobs.pop(0)(), [])
        assert not jobs
        hs = []
        for qb in range(4):
            blk, half = qb // 2, qb % 2
            h = wo_proj(x_ref[blk, 128 * half:128 * half + 128, :].astype(f32), ot0, [qb])
            h_ref[blk, 128 * half:128 * half + 128, :] = h
            hs.append(h)
        xn_ref[...] = pltpu.bitcast(_ln(x_ref[2].astype(f32)).astype(bf16), i32)
        for qb in range(4):
            blk, half = qb // 2, qb % 2
            hn_ref[blk, 64 * half:64 * half + 64, :] = pltpu.bitcast(_ln(hs[qb]).astype(bf16), i32)
        for c in ce:
            c.wait()

    @pl.when(s_id == 2)
    def _():
        xrest().wait()

    @pl.when((s_id > 0) & (s_id < NB - 1))
    def _():
        blk = s_id + 1
        tokens = []
        ffn = FFN(tokens)
        zs = jax.lax.shift_right_logical(s_id, 6)

        def paced(plan):
            zeros = []
            for npass in plan:
                ffn.emit(npass)
                zeros += [pltpu.bitcast(pltpu.bitcast(tk, i32) & zs, f32) for tk in tokens]
            return zeros
        xn = pltpu.bitcast(xn_ref[...], bf16)
        store_qk(False, qk_tiles(xn, 0, 10), blk)
        ffn.emit(10)
        store_vt(xn, blk)
        run_attn(False, 2, blk, 1, [PAT_MID] * 16, ffn, tokens)
        ffn.emit(8)
        h = wo_proj(x_ref[blk].astype(f32), ot1, [0, 1])
        h_ref[blk & 3] = h
        assert ffn.left <= 70
        z2 = paced((4, 4, 4, 4))
        hn_ref[blk & 1] = pltpu.bitcast(_ln(h, z2).astype(bf16), i32)
        z1 = paced((8, 8))
        xn_ref[...] = pltpu.bitcast(_ln(x_ref[jnp.minimum(blk + 1, NB - 1)].astype(f32), z1).astype(bf16), i32)
        ffn.emit(1000)

    @pl.when(s_id >= NB - 1)
    def _():
        FFN([]).emit(1000)

    @pl.when(s_id == NB)
    def _():
        pltpu.make_async_copy(o_ref, o_ref, osem.at[0]).wait()


@jax.jit
def pallas_sequential_preLN__sliding_block__glu_gated_swiglu__prompt_kernel(
    A_x: jax.Array,
    A_wqkv: jax.Array,
    A_wo: jax.Array,
    B_x: jax.Array,
    B_w1: jax.Array,
    B_w3: jax.Array,
    B_w2: jax.Array,
):
    anyspec = pl.BlockSpec(memory_space=pl.ANY)
    out = pl.pallas_call(
        _kernel,
        out_shape=jax.ShapeDtypeStruct((NB, T, D), bf16),
        grid=(NB + 1,),
        in_specs=[anyspec] * 6,
        out_specs=anyspec,
        scratch_shapes=[
            pltpu.VMEM((NB, T, D), bf16),
            pltpu.VMEM((D, 3 * D), bf16),
            pltpu.VMEM((D, D), bf16),
            pltpu.VMEM((D, D), bf16),
            pltpu.VMEM((2, F, D), bf16),
            pltpu.VMEM((F, D), bf16),
            pltpu.VMEM((NG, T, 128), i32),
            pltpu.VMEM((NG, T // 2, 128), i32),
            pltpu.VMEM((NG, (W + S) // 2, 128), i32),
            pltpu.VMEM((2 + S // 128, D // 2, 128), i32),
            pltpu.VMEM((4, D, 128), f32),
            pltpu.VMEM((2, D, 128), f32),
            pltpu.VMEM((1024, 128), f32),
            pltpu.VMEM((1024, 128), f32),
            pltpu.VMEM((1024, 128), f32),
            pltpu.VMEM((4, T, D), f32),
            pltpu.VMEM((2, T // 2, D), i32),
            pltpu.VMEM((T // 2, D), i32),
            pltpu.VMEM((NB, 5, T, 128), bf16),
            pltpu.SemaphoreType.DMA((8,)),
            pltpu.SemaphoreType.DMA((1,)),
        ],
        compiler_params=pltpu.CompilerParams(dimension_semantics=("arbitrary",),
                                             vmem_limit_bytes=100 * 1024 * 1024,
                                             disable_bounds_checks=True),
    )(A_x.reshape(NB, T, D), A_wqkv, A_wo, B_w1.T, B_w3.T, B_w2)
    return out.reshape(1, S, D)
```
